```python
import jax
import jax.numpy as jnp

def _softmax(x, axis=-1):
    return jax.nn.softmax(x, axis=axis)
def _gelu(x):
    return jax.nn.gelu(x, approximate=True)
def _silu(x):
    return jax.nn.silu(x)
def _sigmoid(x):
    return jax.nn.sigmoid(x)
def _layernorm(x, axis=-1, eps=1e-5):
    m = jnp.mean(x, axis=axis, keepdims=True)
    v = jnp.var(x, axis=axis, keepdims=True)
    return (x - m) / jnp.sqrt(v + eps)
def _scatter_add(tgt, idx, src, axis=0):
    return tgt.at[idx].add(src)
def _segment_sum(src, seg, n):
    return jax.ops.segment_sum(src, seg, n)
class _Rng:
    def __init__(self, key):
        self._k = key
    def _next(self):
        self._k, sub = jax.random.split(self._k)
        return sub
    def normal(self, shape):
        return jax.random.normal(self._next(), shape, dtype=jnp.bfloat16)
    def randint(self, lo, hi, shape):
        return jax.random.randint(self._next(), shape, lo, hi, dtype=jnp.int32)
    def uniform(self, shape, lo=0.0, hi=1.0):
        return jax.random.uniform(self._next(), shape, jnp.bfloat16, lo, hi)
    def permutation(self, n):
        return jax.random.permutation(self._next(), n)


kernel_name = 'gated_mix__mha_block_cached__compressed_kv_cla__decode'

def setup_inputs():
    _rng = _Rng(jax.random.key(int.from_bytes(__import__("os").urandom(4), "little")))
    _w = (lambda a: (lambda t: t.astype(jnp.bfloat16) if jnp.issubdtype(t.dtype, jnp.floating) else t)(jnp.asarray(a)))
    def _A_setup():
        B, Sq, D = 2, 1, 512
        H, Sk, Dh = 32, 8192, 128
        return {
            "x": _w((lambda *s: _rng.normal(s) * 0.05)(B, Sq, D)),
            "k_cache": _w((lambda *s: _rng.normal(s) * 0.05)(B, H, Sk, Dh)),
            "v_cache": _w((lambda *s: _rng.normal(s) * 0.05)(B, H, Sk, Dh)),
            "wq": _w((lambda *s: _rng.normal(s) * 0.05)(D, H * Dh) * (D ** -0.5)),
            "wo": _w((lambda *s: _rng.normal(s) * 0.05)(H * Dh, D) * ((H * Dh) ** -0.5)),
        }
    _A_in = _A_setup()

    def _B_setup():
        B, H, Sq, Sk, D, M = 2, 32, 1, 8192, 128, 512
        Dc = 4 * D
        return {
            "x": _w((lambda *s: _rng.normal(s) * 0.05)(B, Sq, M)),
            "c_kv": _w((lambda *s: _rng.normal(s) * 0.05)(B, Sk, Dc)),
            "w_q": _w((lambda *s: _rng.normal(s) * 0.05)(M, H, D) * (M ** -0.5)),
            "w_uk": _w((lambda *s: _rng.normal(s) * 0.05)(Dc, H, D) * (Dc ** -0.5)),
            "w_uv": _w((lambda *s: _rng.normal(s) * 0.05)(Dc, H, D) * (Dc ** -0.5)),
            "w_o": _w((lambda *s: _rng.normal(s) * 0.05)(H, D, M) * ((H * D) ** -0.5)),
        }
    _B_in = _B_setup()

    return {
        "A_x": _A_in["x"],
        "A_k_cache": _A_in["k_cache"],
        "A_v_cache": _A_in["v_cache"],
        "A_wq": _A_in["wq"],
        "A_wo": _A_in["wo"],
        "B_x": _B_in["x"],
        "B_c_kv": _B_in["c_kv"],
        "B_w_q": _B_in["w_q"],
        "B_w_uk": _B_in["w_uk"],
        "B_w_uv": _B_in["w_uv"],
        "B_w_o": _B_in["w_o"],
        "gate_w": _w((lambda *s: _rng.normal(s) * 0.05)(512)),
    }

def reference(A_x, A_k_cache, A_v_cache, A_wq, A_wo, B_x, B_c_kv, B_w_q, B_w_uk, B_w_uv, B_w_o, gate_w):
    def _A_ref(x, k_cache, v_cache, wq, wo):
        B, Sq, D = x.shape
        H, Dh = 32, 128
        q = (lambda x, *d: x.transpose(*d))((x @ wq).reshape(B, Sq, H, Dh), 0, 2, 1, 3)
        scores = jnp.einsum("bhqd,bhkd->bhqk", q, k_cache) * (Dh ** -0.5)
        p = _softmax(scores, axis=-1)
        o = jnp.einsum("bhqk,bhkd->bhqd", p, v_cache)
        return (lambda x, *d: x.transpose(*d))(o, 0, 2, 1, 3).reshape(B, Sq, H * Dh) @ wo

    def _B_ref(x, c_kv, w_q, w_uk, w_uv, w_o):
        B, Sq, M = x.shape[0], x.shape[1], x.shape[2]
        Sk = c_kv.shape[1]
        H, D = w_q.shape[1], w_q.shape[2]
        q = jnp.einsum("bqm,mhd->bhqd", x, w_q)
        k = jnp.einsum("bkc,chd->bhkd", c_kv, w_uk)
        v = jnp.einsum("bkc,chd->bhkd", c_kv, w_uv)
        scores = jnp.einsum("bhqd,bhkd->bhqk", q, k) * (D ** -0.5)
        off = Sk - Sq
        qi = jnp.arange(Sq)[:, None]
        kj = jnp.arange(Sk)[None, :]
        cmask = kj <= (qi + off)
        scores = jnp.where(cmask[None, None], scores, -1e9)
        p = _softmax(scores, axis=-1)
        ctx = jnp.einsum("bhqk,bhkd->bhqd", p, v)
        return jnp.einsum("bhqd,hdm->bqm", ctx, w_o)

    x = A_x
    g = _sigmoid((x * gate_w).sum(-1, keepdims=True))
    a = _A_ref(x, A_k_cache, A_v_cache, A_wq, A_wo)
    b = _B_ref(x, B_c_kv, B_w_q, B_w_uk, B_w_uv, B_w_o)
    return g * a + (1 - g) * b
```

```python
import functools
import jax
import jax.numpy as jnp
import numpy as np
import jax.experimental.pallas as pl
import jax.experimental.pallas.tpu as pltpu

NB, NH, SK, DH, DM, DC = 2, 32, 8192, 128, 512, 512
NBH = NB * NH
ROWS = 16


def _pair_weights(w_ref, hp):
    w32 = w_ref.bitcast(jnp.uint32)
    w = w32[pl.ds(hp, DC, stride=NH // 2), :]
    lo = pltpu.bitcast(w << 16, jnp.float32).astype(jnp.bfloat16)
    hi = pltpu.bitcast(w & jnp.uint32(0xFFFF0000), jnp.float32).astype(jnp.bfloat16)
    return lo, hi


def _make(R=6, NPRE=8):
    scale = DH ** -0.5

    def kernel(x_ref, g_ref, k_hbm, v_hbm, wq_hbm, wo_hbm, c_hbm, wqb_hbm, wuk_hbm, wuv_hbm, wob_hbm,
               out_ref,
               kbuf, vbuf, wq_v, wo_v, c_v, wqb_v, wuk_v, wuv_v, wob_v, q_v, ksem, vsem, wsem):
        def kcopy(i, slot):
            return pltpu.make_async_copy(k_hbm.at[i], kbuf.at[slot], ksem.at[slot])

        def vcopy(i, slot):
            return pltpu.make_async_copy(v_hbm.at[i], vbuf.at[slot], vsem.at[slot])

        c_wq = pltpu.make_async_copy(wq_hbm, wq_v, wsem.at[0])
        c_wqb = pltpu.make_async_copy(wqb_hbm, wqb_v, wsem.at[1])
        c_wuk = pltpu.make_async_copy(wuk_hbm, wuk_v, wsem.at[2])
        c_c0 = pltpu.make_async_copy(c_hbm.at[0], c_v.at[0], wsem.at[3])
        c_c1 = pltpu.make_async_copy(c_hbm.at[1], c_v.at[1], wsem.at[4])
        c_wuv = pltpu.make_async_copy(wuv_hbm, wuv_v, wsem.at[5])
        c_wob = pltpu.make_async_copy(wob_hbm, wob_v, wsem.at[6])
        c_wo = pltpu.make_async_copy(wo_hbm, wo_v, wsem.at[7])

        c_wq.start()
        c_wo.start()
        for s in range(R):
            kcopy(s, s).start()
            vcopy(s, s).start()
        c_wqb.start()
        c_wuk.start()
        c_c0.start()
        c_c1.start()
        c_wuv.start()
        c_wob.start()

        x2 = x_ref[...]
        row16 = jax.lax.broadcasted_iota(jnp.int32, (ROWS, DM), 0)
        xf = x2.astype(jnp.float32)
        x16 = jnp.where(row16 == 0, xf[0:1, :], jnp.where(row16 == 1, xf[1:2, :], 0.0)).astype(jnp.bfloat16)

        c_wq.wait()
        qa = jnp.dot(x16, wq_v[...], preferred_element_type=jnp.float32).astype(jnp.bfloat16)
        for h in range(NH):
            q_v[h] = qa[:, h * DH:(h + 1) * DH]
        c_wo.wait()

        rowh = jax.lax.broadcasted_iota(jnp.int32, (ROWS, DH), 0)

        def head(i, acc):
            h = i % NH
            b = i // NH
            slot = i % R
            kcopy(i, slot).wait()
            q = q_v[h]
            s = jax.lax.dot_general(q, kbuf[slot], (((1,), (1,)), ((), ())),
                                    preferred_element_type=jnp.float32) * scale
            m = jnp.max(s, axis=1, keepdims=True)
            p = jnp.exp(s - m)
            l = jnp.sum(p, axis=1, keepdims=True)
            vcopy(i, slot).wait()
            o = jnp.dot(p.astype(jnp.bfloat16), vbuf[slot], preferred_element_type=jnp.float32)
            o = jnp.where(rowh == b, o / l, 0.0).astype(jnp.bfloat16)
            w = wo_v[pl.ds(pl.multiple_of(h * DH, DH), DH), :]
            acc = acc + jnp.dot(o, w, preferred_element_type=jnp.float32)

            @pl.when(i + R < NBH)
            def _():
                kcopy(i + R, slot).start()
                vcopy(i + R, slot).start()
            return acc

        acc = jnp.zeros((ROWS, DM), jnp.float32)
        acc = jax.lax.fori_loop(0, NPRE, head, acc)

        c_wqb.wait()
        c_wuk.wait()
        rowbh = jax.lax.broadcasted_iota(jnp.int32, (NBH, DH), 0) % NH

        def qabs_body(hp, qacc):
            wq0, wq1 = _pair_weights(wqb_v, hp)
            wk0, wk1 = _pair_weights(wuk_v, hp)
            for j, (wq_h, wk_h) in enumerate(((wq0, wk0), (wq1, wk1))):
                qh = jnp.dot(x16, wq_h, preferred_element_type=jnp.float32)
                qh = qh.astype(jnp.bfloat16).astype(jnp.float32)
                qb = jnp.concatenate([jnp.broadcast_to(qh[0:1, :], (NH, DH)),
                                      jnp.broadcast_to(qh[1:2, :], (NH, DH))], axis=0)
                lhs = jnp.where(rowbh == 2 * hp + j, qb, 0.0).astype(jnp.bfloat16)
                qacc = qacc + jax.lax.dot_general(lhs, wk_h, (((1,), (1,)), ((), ())),
                                                  preferred_element_type=jnp.float32)
            return qacc

        qabs = jnp.zeros((NBH, DC), jnp.float32)
        for hp in range(NH // 2):
            qabs = qabs_body(hp, qabs)
        qabs = qabs.astype(jnp.bfloat16)

        ctx = []
        for b, cp in ((0, c_c0), (1, c_c1)):
            cp.wait()
            c = c_v[b]
            s = jax.lax.dot_general(qabs[b * NH:(b + 1) * NH], c, (((1,), (1,)), ((), ())),
                                    preferred_element_type=jnp.float32) * scale
            m = jnp.max(s, axis=1, keepdims=True)
            p = jnp.exp(s - m)
            l = jnp.sum(p, axis=1, keepdims=True)
            cl = jnp.dot(p.astype(jnp.bfloat16), c, preferred_element_type=jnp.float32)
            ctx.append(cl / l)
        ctxl = jnp.concatenate(ctx, axis=0).astype(jnp.bfloat16)

        c_wuv.wait()
        c_wob.wait()

        def outb_body(hp, oacc):
            wv0, wv1 = _pair_weights(wuv_v, hp)
            for j, wv_h in enumerate((wv0, wv1)):
                r = jnp.dot(ctxl, wv_h, preferred_element_type=jnp.float32)
                r = jnp.where(rowbh == 2 * hp + j, r, 0.0).astype(jnp.bfloat16)
                w = wob_v[pl.ds((2 * hp + j) * DH, DH), :]
                oacc = oacc + jnp.dot(r, w, preferred_element_type=jnp.float32)
            return oacc

        ob = jnp.zeros((NBH, DM), jnp.float32)
        for hp in range(NH // 2):
            ob = outb_body(hp, ob)
        outb0 = jnp.sum(ob[0:NH], axis=0, keepdims=True)
        outb1 = jnp.sum(ob[NH:], axis=0, keepdims=True)
        outb = jnp.where(row16 == 0, outb0, jnp.where(row16 == 1, outb1, 0.0))

        acc = jax.lax.fori_loop(NPRE, NBH, head, acc)

        gsum = jnp.sum(xf * g_ref[...].astype(jnp.float32), axis=1, keepdims=True)
        g = jax.nn.sigmoid(gsum)
        res = g * acc[0:2] + (1.0 - g) * outb[0:2]
        out_ref[...] = res.astype(out_ref.dtype)

    def run(A_x, A_k_cache, A_v_cache, A_wq, A_wo, B_x, B_c_kv, B_w_q, B_w_uk, B_w_uv, B_w_o, gate_w):
        del B_x
        x2 = A_x.reshape(NB, DM)
        g2 = gate_w.reshape(1, DM)
        k3 = A_k_cache.reshape(NBH, SK, DH)
        v3 = A_v_cache.reshape(NBH, SK, DH)
        wqb = B_w_q.reshape(DM * NH, DH)
        wuk = B_w_uk.reshape(DC * NH, DH)
        wuv = B_w_uv.reshape(DC * NH, DH)
        wob = B_w_o.reshape(NH * DH, DM)
        any_spec = pl.BlockSpec(memory_space=pl.ANY)
        vm = pl.BlockSpec(memory_space=pltpu.VMEM)
        bf = jnp.bfloat16
        out = pl.pallas_call(
            kernel,
            in_specs=[vm, vm] + [any_spec] * 9,
            out_specs=vm,
            out_shape=jax.ShapeDtypeStruct((NB, DM), bf),
            scratch_shapes=[
                pltpu.VMEM((R, SK, DH), bf), pltpu.VMEM((R, SK, DH), bf),
                pltpu.VMEM((DM, NH * DH), bf), pltpu.VMEM((NH * DH, DM), bf),
                pltpu.VMEM((NB, SK, DC), bf),
                pltpu.VMEM((DM * NH, DH), bf), pltpu.VMEM((DC * NH, DH), bf), pltpu.VMEM((DC * NH, DH), bf),
                pltpu.VMEM((NH * DH, DM), bf),
                pltpu.VMEM((NH, ROWS, DH), bf),
                pltpu.SemaphoreType.DMA((R,)), pltpu.SemaphoreType.DMA((R,)), pltpu.SemaphoreType.DMA((8,)),
            ],
            compiler_params=pltpu.CompilerParams(vmem_limit_bytes=110 * 1024 * 1024),
        )(x2, g2, k3, v3, A_wq, A_wo, B_c_kv, wqb, wuk, wuv, wob)
        return out.reshape(NB, 1, DM)

    return run


@jax.jit
def pallas_gated_mix__mha_block_cached__compressed_kv_cla__decode_kernel(
    A_x, A_k_cache, A_v_cache, A_wq, A_wo, B_x, B_c_kv, B_w_q, B_w_uk, B_w_uv, B_w_o, gate_w,
):
    return _make()(A_x, A_k_cache, A_v_cache, A_wq, A_wo, B_x, B_c_kv, B_w_q, B_w_uk, B_w_uv, B_w_o, gate_w)
```

```python
import jax
import jax.numpy as jnp
import numpy as np
import jax.experimental.pallas as pl
import jax.experimental.pallas.tpu as pltpu

NB, NH, SK, DH, DM, DC = 2, 32, 8192, 128, 512, 512
NBH = NB * NH
ROWS = 16
NSUB = 4
PER = 16
HALF = SK // 2


def _pair_weights(w_ref, hp):
    w32 = w_ref.bitcast(jnp.uint32)
    w = w32[pl.ds(hp, DC, stride=NH // 2), :]
    lo = pltpu.bitcast(w << 16, jnp.float32).astype(jnp.bfloat16)
    hi = pltpu.bitcast(w & jnp.uint32(0xFFFF0000), jnp.float32).astype(jnp.bfloat16)
    return lo, hi


def _rows_chunk(src, dst, base, nrows):
    def f(c, s):
        r0 = pl.multiple_of(base + (c + s * PER) * nrows, nrows)
        return src.at[pl.ds(r0, nrows)], dst.at[pl.ds(r0, nrows)]
    return f


def _issue_unit(f0, sem0, f1, sem1):
    def body(c, carry):
        for s in range(NSUB):
            a, b = f0(c, s)
            pltpu.make_async_copy(a, b, sem0).start(priority=0)
            a, b = f1(c, s)
            pltpu.make_async_copy(a, b, sem1).start(priority=1)
        return carry
    jax.lax.fori_loop(0, PER, body, 0)


def _wait_all(buf, sem):
    pltpu.make_async_copy(buf, buf, sem).wait()


def _make(R=3):
    scale = DH ** -0.5

    def kernel(x_ref, g_ref, k_hbm, v_hbm, wq_hbm, wo_hbm, c_hbm, wqb_hbm, wuk_hbm, wuv_hbm, wob_hbm,
               out_ref,
               kbuf, vbuf, wq_v, wo_v, c_v, wqb_v, wuk_v, wuv_v, wob_v, q_v, ksem, vsem, wsem):
        def issue_kv(i, slot):
            _issue_unit(_rows_chunk(k_hbm.at[i], kbuf.at[slot], 0, 128), ksem.at[slot],
                        _rows_chunk(v_hbm.at[i], vbuf.at[slot], 0, 128), vsem.at[slot])

        def wq_chunk(u):
            def f(c, s):
                r0 = pl.multiple_of(u * 256 + (c + PER * (s // 2)) * 8, 8)
                sl = (pl.ds(r0, 8), pl.ds((s % 2) * 2048, 2048))
                return wq_hbm.at[sl], wq_v.at[sl]
            return f

        def issue_wq_wo(u):
            _issue_unit(wq_chunk(u), wsem.at[0], _rows_chunk(wo_hbm, wo_v, u * 2048, 32), wsem.at[1])

        def issue_wqb_wuk(u):
            _issue_unit(_rows_chunk(wqb_hbm, wqb_v, u * 8192, 128), wsem.at[2],
                        _rows_chunk(wuk_hbm, wuk_v, u * 8192, 128), wsem.at[3])

        def issue_c(qtr):
            _issue_unit(_rows_chunk(c_hbm.at[0], c_v.at[0], qtr * 2048, 32), wsem.at[4 + qtr // 2],
                        _rows_chunk(c_hbm.at[1], c_v.at[1], qtr * 2048, 32), wsem.at[6 + qtr // 2])

        def issue_wuv_wob(u):
            _issue_unit(_rows_chunk(wuv_hbm, wuv_v, u * 8192, 128), wsem.at[8],
                        _rows_chunk(wob_hbm, wob_v, u * 2048, 32), wsem.at[9])

        issue_wq_wo(0)
        issue_wq_wo(1)
        issue_wqb_wuk(0)

        x2 = x_ref[...]
        row16 = jax.lax.broadcasted_iota(jnp.int32, (ROWS, DM), 0)
        xf = x2.astype(jnp.float32)
        x16 = jnp.where(row16 == 0, xf[0:1, :], jnp.where(row16 == 1, xf[1:2, :], 0.0)).astype(jnp.bfloat16)

        _wait_all(wq_v, wsem.at[0])
        qa = jnp.dot(x16, wq_v[...], preferred_element_type=jnp.float32).astype(jnp.bfloat16)
        for h in range(NH):
            q_v[h] = qa[:, h * DH:(h + 1) * DH]

        issue_wqb_wuk(1)
        gsum = jnp.sum(xf * g_ref[...].astype(jnp.float32), axis=1, keepdims=True)
        g = jax.nn.sigmoid(gsum)
        issue_c(0)

        _wait_all(wqb_v, wsem.at[2])
        _wait_all(wuk_v, wsem.at[3])
        rowbh = jax.lax.broadcasted_iota(jnp.int32, (NBH, DH), 0) % NH

        def qabs_pair(hp, qacc):
            wq0, wq1 = _pair_weights(wqb_v, hp)
            wk0, wk1 = _pair_weights(wuk_v, hp)
            for j, (wq_h, wk_h) in enumerate(((wq0, wk0), (wq1, wk1))):
                qh = jnp.dot(x16, wq_h, preferred_element_type=jnp.float32)
                qh = qh.astype(jnp.bfloat16).astype(jnp.float32)
                qb = jnp.concatenate([jnp.broadcast_to(qh[0:1, :], (NH, DH)),
                                      jnp.broadcast_to(qh[1:2, :], (NH, DH))], axis=0)
                lhs = jnp.where(rowbh == 2 * hp + j, qb, 0.0).astype(jnp.bfloat16)
                qacc = qacc + jax.lax.dot_general(lhs, wk_h, (((1,), (1,)), ((), ())),
                                                  preferred_element_type=jnp.float32)
            return qacc

        qabs = jnp.zeros((NBH, DC), jnp.float32)
        for hp in range(0, NH // 4):
            qabs = qabs_pair(hp, qabs)
        issue_c(1)
        for hp in range(NH // 4, NH // 2):
            qabs = qabs_pair(hp, qabs)
        qabs = qabs.astype(jnp.bfloat16)
        issue_c(2)

        def b_half(b, hf):
            _wait_all(c_v.at[b, pl.ds(hf * HALF, HALF)], wsem.at[4 + 2 * b + hf])
            c = c_v[b, pl.ds(hf * HALF, HALF), :]
            s = jax.lax.dot_general(qabs[b * NH:(b + 1) * NH], c, (((1,), (1,)), ((), ())),
                                    preferred_element_type=jnp.float32) * scale
            m = jnp.max(s, axis=1, keepdims=True)
            p = jnp.exp(s - m)
            l = jnp.sum(p, axis=1, keepdims=True)
            cl = jnp.dot(p.astype(jnp.bfloat16), c, preferred_element_type=jnp.float32)
            return m, l, cl

        def merge(h0, h1):
            m0, l0, c0 = h0
            m1, l1, c1 = h1
            m = jnp.maximum(m0, m1)
            a0 = jnp.exp(m0 - m)
            a1 = jnp.exp(m1 - m)
            return (a0 * c0 + a1 * c1) / (a0 * l0 + a1 * l1)

        p00 = b_half(0, 0)
        issue_c(3)
        p10 = b_half(1, 0)
        issue_wuv_wob(0)
        p01 = b_half(0, 1)
        issue_wuv_wob(1)
        p11 = b_half(1, 1)
        ctxl = jnp.concatenate([merge(p00, p01), merge(p10, p11)], axis=0).astype(jnp.bfloat16)
        issue_kv(0, 0)

        _wait_all(wuv_v, wsem.at[8])
        _wait_all(wob_v, wsem.at[9])

        def outb_pair(hp, oacc):
            wv0, wv1 = _pair_weights(wuv_v, hp)
            for j, wv_h in enumerate((wv0, wv1)):
                r = jnp.dot(ctxl, wv_h, preferred_element_type=jnp.float32)
                r = jnp.where(rowbh == 2 * hp + j, r, 0.0).astype(jnp.bfloat16)
                w = wob_v[pl.ds((2 * hp + j) * DH, DH), :]
                oacc = oacc + jnp.dot(r, w, preferred_element_type=jnp.float32)
            return oacc

        ob = jnp.zeros((NBH, DM), jnp.float32)
        for hp in range(0, NH // 4):
            ob = outb_pair(hp, ob)
        issue_kv(1, 1)
        for hp in range(NH // 4, NH // 2):
            ob = outb_pair(hp, ob)
        outb0 = jnp.sum(ob[0:NH], axis=0, keepdims=True)
        outb1 = jnp.sum(ob[NH:], axis=0, keepdims=True)
        outb = jnp.where(row16 == 0, outb0, jnp.where(row16 == 1, outb1, 0.0))
        for s_ in range(2, R):
            issue_kv(s_, s_)

        _wait_all(wo_v, wsem.at[1])
        rowh = jax.lax.broadcasted_iota(jnp.int32, (ROWS, DH), 0)

        def head(i, acc):
            h = i % NH
            b = i // NH
            slot = i % R
            _wait_all(kbuf.at[slot], ksem.at[slot])
            q = q_v[h]
            s = jax.lax.dot_general(q, kbuf[slot], (((1,), (1,)), ((), ())),
                                    preferred_element_type=jnp.float32) * scale
            m = jnp.max(s, axis=1, keepdims=True)
            p = jnp.exp(s - m)
            l = jnp.sum(p, axis=1, keepdims=True)
            _wait_all(vbuf.at[slot], vsem.at[slot])
            o = jnp.dot(p.astype(jnp.bfloat16), vbuf[slot], preferred_element_type=jnp.float32)
            o = jnp.where(rowh == b, o / l, 0.0).astype(jnp.bfloat16)
            w = wo_v[pl.ds(pl.multiple_of(h * DH, DH), DH), :]
            acc = acc + jnp.dot(o, w, preferred_element_type=jnp.float32)

            @pl.when(i + R < NBH)
            def _():
                issue_kv(i + R, slot)
            return acc

        acc = jax.lax.fori_loop(0, NBH, head, jnp.zeros((ROWS, DM), jnp.float32))
        res = g * acc[0:2] + (1.0 - g) * outb[0:2]
        out_ref[...] = res.astype(out_ref.dtype)

    def run(A_x, A_k_cache, A_v_cache, A_wq, A_wo, B_x, B_c_kv, B_w_q, B_w_uk, B_w_uv, B_w_o, gate_w):
        del B_x
        x2 = A_x.reshape(NB, DM)
        g2 = gate_w.reshape(1, DM)
        k3 = A_k_cache.reshape(NBH, SK, DH)
        v3 = A_v_cache.reshape(NBH, SK, DH)
        wqb = B_w_q.reshape(DM * NH, DH)
        wuk = B_w_uk.reshape(DC * NH, DH)
        wuv = B_w_uv.reshape(DC * NH, DH)
        wob = B_w_o.reshape(NH * DH, DM)
        any_spec = pl.BlockSpec(memory_space=pl.ANY)
        vm = pl.BlockSpec(memory_space=pltpu.VMEM)
        bf = jnp.bfloat16
        out = pl.pallas_call(
            kernel,
            in_specs=[vm, vm] + [any_spec] * 9,
            out_specs=vm,
            out_shape=jax.ShapeDtypeStruct((NB, DM), bf),
            scratch_shapes=[
                pltpu.VMEM((R, SK, DH), bf), pltpu.VMEM((R, SK, DH), bf),
                pltpu.VMEM((DM, NH * DH), bf), pltpu.VMEM((NH * DH, DM), bf),
                pltpu.VMEM((NB, SK, DC), bf),
                pltpu.VMEM((DM * NH, DH), bf), pltpu.VMEM((DC * NH, DH), bf), pltpu.VMEM((DC * NH, DH), bf),
                pltpu.VMEM((NH * DH, DM), bf),
                pltpu.VMEM((NH, ROWS, DH), bf),
                pltpu.SemaphoreType.DMA((R,)), pltpu.SemaphoreType.DMA((R,)), pltpu.SemaphoreType.DMA((10,)),
            ],
            compiler_params=pltpu.CompilerParams(vmem_limit_bytes=110 * 1024 * 1024),
        )(x2, g2, k3, v3, A_wq, A_wo, B_c_kv, wqb, wuk, wuv, wob)
        return out.reshape(NB, 1, DM)

    return run


@jax.jit
def pallas_gated_mix__mha_block_cached__compressed_kv_cla__decode_kernel(
    A_x, A_k_cache, A_v_cache, A_wq, A_wo, B_x, B_c_kv, B_w_q, B_w_uk, B_w_uv, B_w_o, gate_w,
):
    return _make(R=3)(A_x, A_k_cache, A_v_cache, A_wq, A_wo, B_x, B_c_kv, B_w_q, B_w_uk, B_w_uv, B_w_o, gate_w)
```

```python
import jax
import jax.numpy as jnp
import numpy as np
import jax.experimental.pallas as pl
import jax.experimental.pallas.tpu as pltpu

NB, NH, SK, DH, DM, DC = 2, 32, 8192, 128, 512, 512
NBH = NB * NH
ROWS = 16
NSUB = 4
PER = 16
HALF = SK // 2


def _pair_weights(w_ref, hp):
    w32 = w_ref.bitcast(jnp.uint32)
    w = w32[pl.ds(hp, DC, stride=NH // 2), :]
    lo = pltpu.bitcast(w << 16, jnp.float32).astype(jnp.bfloat16)
    hi = pltpu.bitcast(w & jnp.uint32(0xFFFF0000), jnp.float32).astype(jnp.bfloat16)
    return lo, hi


def _rows_chunk(src, dst, base, nrows):
    def f(c, s):
        r0 = pl.multiple_of(base + (c + s * PER) * nrows, nrows)
        return src.at[pl.ds(r0, nrows)], dst.at[pl.ds(r0, nrows)]
    return f


def _issue_unit(f0, sem0, f1, sem1):
    def body(c, carry):
        for s in range(NSUB):
            a, b = f0(c, s)
            pltpu.make_async_copy(a, b, sem0).start(priority=0)
            a, b = f1(c, s)
            pltpu.make_async_copy(a, b, sem1).start(priority=1)
        return carry
    jax.lax.fori_loop(0, PER, body, 0)


def _wait_all(buf, sem):
    pltpu.make_async_copy(buf, buf, sem).wait()


def _make(R=3):
    scale = DH ** -0.5

    def kernel(x_hbm, g_hbm, k_hbm, v_hbm, wq_hbm, wo_hbm, c_hbm, wqb_hbm, wuk_hbm, wuv_hbm, wob_hbm,
               out_ref,
               kbuf, vbuf, wq_v, wo_v, c_v, wqb_v, wuk_v, wuv_v, wob_v, q_v, x_v, g_v, ksem, vsem, wsem):
        def issue_kv(i, slot):
            _issue_unit(_rows_chunk(k_hbm.at[i], kbuf.at[slot], 0, 128), ksem.at[slot],
                        _rows_chunk(v_hbm.at[i], vbuf.at[slot], 0, 128), vsem.at[slot])

        def wq_chunk(u):
            def f(c, s):
                r0 = pl.multiple_of(u * 256 + (c + PER * (s // 2)) * 8, 8)
                sl = (pl.ds(r0, 8), pl.ds((s % 2) * 2048, 2048))
                return wq_hbm.at[sl], wq_v.at[sl]
            return f

        def issue_wq_wo(u):
            _issue_unit(wq_chunk(u), wsem.at[0], _rows_chunk(wo_hbm, wo_v, u * 2048, 32), wsem.at[1])

        def issue_wqb_wuk(u):
            _issue_unit(_rows_chunk(wqb_hbm, wqb_v, u * 8192, 128), wsem.at[2],
                        _rows_chunk(wuk_hbm, wuk_v, u * 8192, 128), wsem.at[3])

        def issue_c(qtr):
            _issue_unit(_rows_chunk(c_hbm.at[0], c_v.at[0], qtr * 2048, 32), wsem.at[4 + qtr // 2],
                        _rows_chunk(c_hbm.at[1], c_v.at[1], qtr * 2048, 32), wsem.at[6 + qtr // 2])

        def issue_wuv_wob(u):
            _issue_unit(_rows_chunk(wuv_hbm, wuv_v, u * 8192, 128), wsem.at[8],
                        _rows_chunk(wob_hbm, wob_v, u * 2048, 32), wsem.at[9])

        cx = pltpu.make_async_copy(x_hbm, x_v, wsem.at[10])
        cg = pltpu.make_async_copy(g_hbm, g_v, wsem.at[11])
        cx.start()
        cg.start()
        issue_wqb_wuk(0)
        issue_wqb_wuk(1)
        issue_c(0)

        cx.wait()
        cg.wait()
        x2 = x_v[...]
        row16 = jax.lax.broadcasted_iota(jnp.int32, (ROWS, DM), 0)
        xf = x2.astype(jnp.float32)
        x16 = jnp.where(row16 == 0, xf[0:1, :], jnp.where(row16 == 1, xf[1:2, :], 0.0)).astype(jnp.bfloat16)
        rowbh = jax.lax.broadcasted_iota(jnp.int32, (NBH, DH), 0) % NH

        def qabs_pair(hp, qacc):
            wq0, wq1 = _pair_weights(wqb_v, hp)
            wk0, wk1 = _pair_weights(wuk_v, hp)
            for j, (wq_h, wk_h) in enumerate(((wq0, wk0), (wq1, wk1))):
                qh = jnp.dot(x16, wq_h, preferred_element_type=jnp.float32)
                qh = qh.astype(jnp.bfloat16).astype(jnp.float32)
                qb = jnp.concatenate([jnp.broadcast_to(qh[0:1, :], (NH, DH)),
                                      jnp.broadcast_to(qh[1:2, :], (NH, DH))], axis=0)
                lhs = jnp.where(rowbh == 2 * hp + j, qb, 0.0).astype(jnp.bfloat16)
                qacc = qacc + jax.lax.dot_general(lhs, wk_h, (((1,), (1,)), ((), ())),
                                                  preferred_element_type=jnp.float32)
            return qacc

        def b_half(b, hf, qabs):
            _wait_all(c_v.at[b, pl.ds(hf * HALF, HALF)], wsem.at[4 + 2 * b + hf])
            c = c_v[b, pl.ds(hf * HALF, HALF), :]
            s = jax.lax.dot_general(qabs[b * NH:(b + 1) * NH], c, (((1,), (1,)), ((), ())),
                                    preferred_element_type=jnp.float32) * scale
            m = jnp.max(s, axis=1, keepdims=True)
            p = jnp.exp(s - m)
            l = jnp.sum(p, axis=1, keepdims=True)
            cl = jnp.dot(p.astype(jnp.bfloat16), c, preferred_element_type=jnp.float32)
            return m, l, cl

        def merge(h0, h1):
            m0, l0, c0 = h0
            m1, l1, c1 = h1
            m = jnp.maximum(m0, m1)
            a0 = jnp.exp(m0 - m)
            a1 = jnp.exp(m1 - m)
            return (a0 * c0 + a1 * c1) / (a0 * l0 + a1 * l1)

        def outb_pair(hp, oacc, ctxl):
            wv0, wv1 = _pair_weights(wuv_v, hp)
            for j, wv_h in enumerate((wv0, wv1)):
                r = jnp.dot(ctxl, wv_h, preferred_element_type=jnp.float32)
                r = jnp.where(rowbh == 2 * hp + j, r, 0.0).astype(jnp.bfloat16)
                w = wob_v[pl.ds((2 * hp + j) * DH, DH), :]
                oacc = oacc + jnp.dot(r, w, preferred_element_type=jnp.float32)
            return oacc

        _wait_all(wqb_v, wsem.at[2])
        _wait_all(wuk_v, wsem.at[3])
        qabs = jnp.zeros((NBH, DC), jnp.float32)
        for hp in range(0, 4):
            qabs = qabs_pair(hp, qabs)
        issue_c(1)
        for hp in range(4, 8):
            qabs = qabs_pair(hp, qabs)
        issue_c(2)
        for hp in range(8, 12):
            qabs = qabs_pair(hp, qabs)
        issue_c(3)
        for hp in range(12, 16):
            qabs = qabs_pair(hp, qabs)
        qabs = qabs.astype(jnp.bfloat16)
        issue_wuv_wob(0)
        p00 = b_half(0, 0, qabs)
        issue_wuv_wob(1)
        p10 = b_half(1, 0, qabs)
        issue_wq_wo(0)
        p01 = b_half(0, 1, qabs)
        issue_wq_wo(1)
        p11 = b_half(1, 1, qabs)
        ctxl = jnp.concatenate([merge(p00, p01), merge(p10, p11)], axis=0).astype(jnp.bfloat16)
        issue_kv(0, 0)

        _wait_all(wuv_v, wsem.at[8])
        _wait_all(wob_v, wsem.at[9])
        ob = jnp.zeros((NBH, DM), jnp.float32)
        for hp in range(0, 6):
            ob = outb_pair(hp, ob, ctxl)
        issue_kv(1, 1)
        for hp in range(6, 12):
            ob = outb_pair(hp, ob, ctxl)
        issue_kv(2, 2)
        for hp in range(12, 16):
            ob = outb_pair(hp, ob, ctxl)
        outb0 = jnp.sum(ob[0:NH], axis=0, keepdims=True)
        outb1 = jnp.sum(ob[NH:], axis=0, keepdims=True)
        outb = jnp.where(row16 == 0, outb0, jnp.where(row16 == 1, outb1, 0.0))
        _wait_all(wq_v, wsem.at[0])
        qa = jnp.dot(x16, wq_v[...], preferred_element_type=jnp.float32).astype(jnp.bfloat16)
        for h in range(NH):
            q_v[h] = qa[:, h * DH:(h + 1) * DH]
        gsum = jnp.sum(xf * g_v[...].reshape(1, DM).astype(jnp.float32), axis=1, keepdims=True)
        g = jax.nn.sigmoid(gsum)
        for s_ in range(3, R):
            issue_kv(s_, s_)

        _wait_all(wo_v, wsem.at[1])
        rowh = jax.lax.broadcasted_iota(jnp.int32, (ROWS, DH), 0)

        def head(i, acc):
            h = i % NH
            b = i // NH
            slot = i % R
            _wait_all(kbuf.at[slot], ksem.at[slot])
            q = q_v[h]
            s = jax.lax.dot_general(q, kbuf[slot], (((1,), (1,)), ((), ())),
                                    preferred_element_type=jnp.float32) * scale
            m = jnp.max(s, axis=1, keepdims=True)
            p = jnp.exp(s - m)
            l = jnp.sum(p, axis=1, keepdims=True)
            _wait_all(vbuf.at[slot], vsem.at[slot])
            o = jnp.dot(p.astype(jnp.bfloat16), vbuf[slot], preferred_element_type=jnp.float32)
            o = jnp.where(rowh == b, o / l, 0.0).astype(jnp.bfloat16)
            w = wo_v[pl.ds(pl.multiple_of(h * DH, DH), DH), :]
            acc = acc + jnp.dot(o, w, preferred_element_type=jnp.float32)

            @pl.when(i + R < NBH)
            def _():
                issue_kv(i + R, slot)
            return acc

        acc = jax.lax.fori_loop(0, NBH, head, jnp.zeros((ROWS, DM), jnp.float32))
        res = g * acc[0:2] + (1.0 - g) * outb[0:2]
        out_ref[...] = res.astype(out_ref.dtype)

    def run(A_x, A_k_cache, A_v_cache, A_wq, A_wo, B_x, B_c_kv, B_w_q, B_w_uk, B_w_uv, B_w_o, gate_w):
        del B_x
        x2 = A_x.reshape(NB, DM)
        k3 = A_k_cache.reshape(NBH, SK, DH)
        v3 = A_v_cache.reshape(NBH, SK, DH)
        wqb = B_w_q.reshape(DM * NH, DH)
        wuk = B_w_uk.reshape(DC * NH, DH)
        wuv = B_w_uv.reshape(DC * NH, DH)
        wob = B_w_o.reshape(NH * DH, DM)
        any_spec = pl.BlockSpec(memory_space=pl.ANY)
        vm = pl.BlockSpec(memory_space=pltpu.VMEM)
        bf = jnp.bfloat16
        out = pl.pallas_call(
            kernel,
            in_specs=[any_spec] * 11,
            out_specs=vm,
            out_shape=jax.ShapeDtypeStruct((NB, DM), bf),
            scratch_shapes=[
                pltpu.VMEM((R, SK, DH), bf), pltpu.VMEM((R, SK, DH), bf),
                pltpu.VMEM((DM, NH * DH), bf), pltpu.VMEM((NH * DH, DM), bf),
                pltpu.VMEM((NB, SK, DC), bf),
                pltpu.VMEM((DM * NH, DH), bf), pltpu.VMEM((DC * NH, DH), bf), pltpu.VMEM((DC * NH, DH), bf),
                pltpu.VMEM((NH * DH, DM), bf),
                pltpu.VMEM((NH, ROWS, DH), bf),
                pltpu.VMEM((NB, DM), bf), pltpu.VMEM((DM,), bf),
                pltpu.SemaphoreType.DMA((R,)), pltpu.SemaphoreType.DMA((R,)), pltpu.SemaphoreType.DMA((12,)),
            ],
            compiler_params=pltpu.CompilerParams(vmem_limit_bytes=110 * 1024 * 1024),
        )(x2, gate_w, k3, v3, A_wq, A_wo, B_c_kv, wqb, wuk, wuv, wob)
        return out.reshape(NB, 1, DM)

    return run


@jax.jit
def pallas_gated_mix__mha_block_cached__compressed_kv_cla__decode_kernel(
    A_x, A_k_cache, A_v_cache, A_wq, A_wo, B_x, B_c_kv, B_w_q, B_w_uk, B_w_uv, B_w_o, gate_w,
):
    return _make(R=3)(A_x, A_k_cache, A_v_cache, A_wq, A_wo, B_x, B_c_kv, B_w_q, B_w_uk, B_w_uv, B_w_o, gate_w)
```

```python
import jax
import jax.numpy as jnp
import numpy as np
import jax.experimental.pallas as pl
import jax.experimental.pallas.tpu as pltpu

NB, NH, SK, DH, DM, DC = 2, 32, 8192, 128, 512, 512
NBH = NB * NH
ROWS = 16
NSUB = 4
PER = 16
HALF = SK // 2


def _pair_weights(w_ref, hp):
    w32 = w_ref.bitcast(jnp.uint32)
    w = w32[pl.ds(hp, DC, stride=NH // 2), :]
    lo = pltpu.bitcast(w << 16, jnp.float32).astype(jnp.bfloat16)
    hi = pltpu.bitcast(w & jnp.uint32(0xFFFF0000), jnp.float32).astype(jnp.bfloat16)
    return lo, hi


def _rows_chunk(src, dst, base, nrows):
    def f(c, s):
        r0 = pl.multiple_of(base + (c + s * PER) * nrows, nrows)
        return src.at[pl.ds(r0, nrows)], dst.at[pl.ds(r0, nrows)]
    return f


def _issue_unit(f0, sem0, f1, sem1, c0=0, c1=PER):
    def body(c, carry):
        for s in range(NSUB):
            a, b = f0(c, s)
            pltpu.make_async_copy(a, b, sem0).start(priority=0)
            a, b = f1(c, s)
            pltpu.make_async_copy(a, b, sem1).start(priority=1)
        return carry
    jax.lax.fori_loop(c0, c1, body, 0)


def _wait_all(buf, sem):
    pltpu.make_async_copy(buf, buf, sem).wait()


def _make(R=3):
    scale = DH ** -0.5

    def kernel(x_hbm, g_hbm, k_hbm, v_hbm, wq_hbm, wo_hbm, c_hbm, wqb_hbm, wuk_hbm, wuv_hbm, wob_hbm,
               out_ref,
               kbuf, vbuf, wq_v, wo_v, c_v, wqb_v, wuk_v, wuv_v, wob_v, q_v, x_v, g_v, oa_v, cb_v, ksem, vsem, wsem):
        def issue_kv(i, slot, c0=0, c1=PER):
            _issue_unit(_rows_chunk(k_hbm.at[i], kbuf.at[slot], 0, 128), ksem.at[slot],
                        _rows_chunk(v_hbm.at[i], vbuf.at[slot], 0, 128), vsem.at[slot], c0, c1)

        def wq_chunk(u):
            def f(c, s):
                r0 = pl.multiple_of(u * 256 + (c + PER * (s // 2)) * 8, 8)
                sl = (pl.ds(r0, 8), pl.ds((s % 2) * 2048, 2048))
                return wq_hbm.at[sl], wq_v.at[sl]
            return f

        def issue_wq_wuv(u):
            _issue_unit(wq_chunk(u), wsem.at[0], _rows_chunk(wuv_hbm, wuv_v, u * 8192, 128), wsem.at[8])

        def issue_wo_wob(u):
            _issue_unit(_rows_chunk(wo_hbm, wo_v, u * 2048, 32), wsem.at[1 + 11 * u],
                        _rows_chunk(wob_hbm, wob_v, u * 2048, 32), wsem.at[9 + 4 * u])

        def issue_wqb_wuk(u):
            _issue_unit(_rows_chunk(wqb_hbm, wqb_v, u * 8192, 128), wsem.at[2],
                        _rows_chunk(wuk_hbm, wuk_v, u * 8192, 128), wsem.at[3])

        def issue_c(qtr):
            _issue_unit(_rows_chunk(c_hbm.at[0], c_v.at[0], qtr * 2048, 32), wsem.at[4 + qtr // 2],
                        _rows_chunk(c_hbm.at[1], c_v.at[1], qtr * 2048, 32), wsem.at[6 + qtr // 2])

        cx = pltpu.make_async_copy(x_hbm, x_v, wsem.at[10])
        cg = pltpu.make_async_copy(g_hbm, g_v, wsem.at[11])
        cx.start()
        cg.start()
        issue_wqb_wuk(0)
        issue_wqb_wuk(1)
        issue_c(0)

        cx.wait()
        cg.wait()
        x2 = x_v[...]
        row16 = jax.lax.broadcasted_iota(jnp.int32, (ROWS, DM), 0)
        xf = x2.astype(jnp.float32)
        x16 = jnp.where(row16 == 0, xf[0:1, :], jnp.where(row16 == 1, xf[1:2, :], 0.0)).astype(jnp.bfloat16)
        rowbh = jax.lax.broadcasted_iota(jnp.int32, (NBH, DH), 0) % NH

        def qabs_pair(hp, qacc):
            wq0, wq1 = _pair_weights(wqb_v, hp)
            wk0, wk1 = _pair_weights(wuk_v, hp)
            for j, (wq_h, wk_h) in enumerate(((wq0, wk0), (wq1, wk1))):
                qh = jnp.dot(x16, wq_h, preferred_element_type=jnp.float32)
                qh = qh.astype(jnp.bfloat16).astype(jnp.float32)
                qb = jnp.concatenate([jnp.broadcast_to(qh[0:1, :], (NH, DH)),
                                      jnp.broadcast_to(qh[1:2, :], (NH, DH))], axis=0)
                lhs = jnp.where(rowbh == 2 * hp + j, qb, 0.0).astype(jnp.bfloat16)
                qacc = qacc + jax.lax.dot_general(lhs, wk_h, (((1,), (1,)), ((), ())),
                                                  preferred_element_type=jnp.float32)
            return qacc

        def b_half(b, hf, qabs):
            _wait_all(c_v.at[b, pl.ds(hf * HALF, HALF)], wsem.at[4 + 2 * b + hf])
            c = c_v[b, pl.ds(hf * HALF, HALF), :]
            s = jax.lax.dot_general(qabs[b * NH:(b + 1) * NH], c, (((1,), (1,)), ((), ())),
                                    preferred_element_type=jnp.float32) * scale
            m = jnp.max(s, axis=1, keepdims=True)
            p = jnp.exp(s - m)
            l = jnp.sum(p, axis=1, keepdims=True)
            cl = jnp.dot(p.astype(jnp.bfloat16), c, preferred_element_type=jnp.float32)
            return m, l, cl

        def merge(h0, h1):
            m0, l0, c0 = h0
            m1, l1, c1 = h1
            m = jnp.maximum(m0, m1)
            a0 = jnp.exp(m0 - m)
            a1 = jnp.exp(m1 - m)
            return (a0 * c0 + a1 * c1) / (a0 * l0 + a1 * l1)

        def ctx_pair(hp, ctxl):
            wv0, wv1 = _pair_weights(wuv_v, hp)
            for j, wv_h in enumerate((wv0, wv1)):
                h = 2 * hp + j
                lhs = jnp.where(row16 == 0, ctxl[h:h + 1, :],
                                jnp.where(row16 == 1, ctxl[NH + h:NH + h + 1, :], 0.0)).astype(jnp.bfloat16)
                r = jnp.dot(lhs, wv_h, preferred_element_type=jnp.float32)
                cb_v[:, h * DH:(h + 1) * DH] = r.astype(jnp.bfloat16)

        _wait_all(wqb_v, wsem.at[2])
        _wait_all(wuk_v, wsem.at[3])
        qabs = jnp.zeros((NBH, DC), jnp.float32)
        for hp in range(0, 4):
            qabs = qabs_pair(hp, qabs)
        issue_c(1)
        for hp in range(4, 8):
            qabs = qabs_pair(hp, qabs)
        issue_c(2)
        for hp in range(8, 12):
            qabs = qabs_pair(hp, qabs)
        issue_c(3)
        for hp in range(12, 16):
            qabs = qabs_pair(hp, qabs)
        qabs = qabs.astype(jnp.bfloat16)
        issue_wq_wuv(0)
        p00 = b_half(0, 0, qabs)
        issue_wq_wuv(1)
        p10 = b_half(1, 0, qabs)
        issue_kv(0, 0, 0, PER // 2)
        p01 = b_half(0, 1, qabs)
        issue_kv(0, 0, PER // 2, PER)
        p11 = b_half(1, 1, qabs)
        ctxl = jnp.concatenate([merge(p00, p01), merge(p10, p11)], axis=0)
        ctxl = ctxl.astype(jnp.bfloat16).astype(jnp.float32)
        issue_kv(1, 1, 0, PER // 2)
        _wait_all(wuv_v, wsem.at[8])
        _wait_all(wq_v, wsem.at[0])
        for hp in range(0, 8):
            ctx_pair(hp, ctxl)
        issue_kv(1, 1, PER // 2, PER)
        for hp in range(8, 16):
            ctx_pair(hp, ctxl)
        issue_kv(2, 2, 0, PER // 2)
        qa = jnp.dot(x16, wq_v[...], preferred_element_type=jnp.float32).astype(jnp.bfloat16)
        for h in range(NH):
            q_v[h] = qa[:, h * DH:(h + 1) * DH]
        gsum = jnp.sum(xf * g_v[...].reshape(1, DM).astype(jnp.float32), axis=1, keepdims=True)
        g = jax.nn.sigmoid(gsum)
        issue_kv(2, 2, PER // 2, PER)

        def head(i, carry):
            h = i % NH
            b = i // NH
            slot = i % R
            _wait_all(kbuf.at[slot], ksem.at[slot])
            s = jax.lax.dot_general(q_v[h], kbuf[slot], (((1,), (1,)), ((), ())),
                                    preferred_element_type=jnp.float32) * scale
            m = jnp.max(s, axis=1, keepdims=True)
            p = jnp.exp(s - m)
            l = jnp.sum(p, axis=1, keepdims=True)
            _wait_all(vbuf.at[slot], vsem.at[slot])
            o = jnp.dot(p.astype(jnp.bfloat16), vbuf[slot], preferred_element_type=jnp.float32)
            oa_v[b, :, pl.ds(pl.multiple_of(h * DH, DH), DH)] = (o / l).astype(jnp.bfloat16)

            @pl.when(i + R < NBH)
            def _():
                issue_kv(i + R, slot)

            @pl.when(i == NBH - R)
            def _():
                issue_wo_wob(0)

            @pl.when(i == NBH - R + 1)
            def _():
                issue_wo_wob(1)
            return carry

        jax.lax.fori_loop(0, NBH, head, 0)

        rowo = jax.lax.broadcasted_iota(jnp.int32, (ROWS, NH * DH), 0)
        oa = jnp.where(rowo == 0, oa_v[0], jnp.where(rowo == 1, oa_v[1], jnp.zeros((), jnp.bfloat16)))
        cb = cb_v[...]
        acc_a = acc_b = None
        HC = NH * DH // 2
        for u in range(2):
            rs = pl.ds(u * HC, HC)
            _wait_all(wo_v.at[rs], wsem.at[1 + 11 * u])
            _wait_all(wob_v.at[rs], wsem.at[9 + 4 * u])
            da = jnp.dot(oa[:, u * HC:(u + 1) * HC], wo_v[rs, :], preferred_element_type=jnp.float32)
            db = jnp.dot(cb[:, u * HC:(u + 1) * HC], wob_v[rs, :], preferred_element_type=jnp.float32)
            acc_a = da if acc_a is None else acc_a + da
            acc_b = db if acc_b is None else acc_b + db
        res = g * acc_a[0:2] + (1.0 - g) * acc_b[0:2]
        out_ref[...] = res.astype(out_ref.dtype)

    def run(A_x, A_k_cache, A_v_cache, A_wq, A_wo, B_x, B_c_kv, B_w_q, B_w_uk, B_w_uv, B_w_o, gate_w):
        del B_x
        x2 = A_x.reshape(NB, DM)
        k3 = A_k_cache.reshape(NBH, SK, DH)
        v3 = A_v_cache.reshape(NBH, SK, DH)
        wqb = B_w_q.reshape(DM * NH, DH)
        wuk = B_w_uk.reshape(DC * NH, DH)
        wuv = B_w_uv.reshape(DC * NH, DH)
        wob = B_w_o.reshape(NH * DH, DM)
        any_spec = pl.BlockSpec(memory_space=pl.ANY)
        vm = pl.BlockSpec(memory_space=pltpu.VMEM)
        bf = jnp.bfloat16
        out = pl.pallas_call(
            kernel,
            in_specs=[any_spec] * 11,
            out_specs=vm,
            out_shape=jax.ShapeDtypeStruct((NB, DM), bf),
            scratch_shapes=[
                pltpu.VMEM((R, SK, DH), bf), pltpu.VMEM((R, SK, DH), bf),
                pltpu.VMEM((DM, NH * DH), bf), pltpu.VMEM((NH * DH, DM), bf),
                pltpu.VMEM((NB, SK, DC), bf),
                pltpu.VMEM((DM * NH, DH), bf), pltpu.VMEM((DC * NH, DH), bf), pltpu.VMEM((DC * NH, DH), bf),
                pltpu.VMEM((NH * DH, DM), bf),
                pltpu.VMEM((NH, ROWS, DH), bf),
                pltpu.VMEM((NB, DM), bf), pltpu.VMEM((DM,), bf),
                pltpu.VMEM((NB, ROWS, NH * DH), bf), pltpu.VMEM((ROWS, NH * DH), bf),
                pltpu.SemaphoreType.DMA((R,)), pltpu.SemaphoreType.DMA((R,)), pltpu.SemaphoreType.DMA((14,)),
            ],
            compiler_params=pltpu.CompilerParams(vmem_limit_bytes=110 * 1024 * 1024),
        )(x2, gate_w, k3, v3, A_wq, A_wo, B_c_kv, wqb, wuk, wuv, wob)
        return out.reshape(NB, 1, DM)

    return run


@jax.jit
def pallas_gated_mix__mha_block_cached__compressed_kv_cla__decode_kernel(
    A_x, A_k_cache, A_v_cache, A_wq, A_wo, B_x, B_c_kv, B_w_q, B_w_uk, B_w_uv, B_w_o, gate_w,
):
    return _make(R=3)(A_x, A_k_cache, A_v_cache, A_wq, A_wo, B_x, B_c_kv, B_w_q, B_w_uk, B_w_uv, B_w_o, gate_w)
```

```python
import jax
import jax.numpy as jnp
import numpy as np
import jax.experimental.pallas as pl
import jax.experimental.pallas.tpu as pltpu

NB, NH, SK, DH, DM, DC = 2, 32, 8192, 128, 512, 512
NBH = NB * NH
ROWS = 16
NSUB = 4
PER = 16
HALF = SK // 2


def _pair_weights(w_ref, hp):
    w32 = w_ref.bitcast(jnp.uint32)
    w = w32[pl.ds(hp, DC, stride=NH // 2), :]
    lo = pltpu.bitcast(w << 16, jnp.float32).astype(jnp.bfloat16)
    hi = pltpu.bitcast(w & jnp.uint32(0xFFFF0000), jnp.float32).astype(jnp.bfloat16)
    return lo, hi


def _rows_chunk(src, dst, base, nrows, per=PER):
    def f(c, s):
        r0 = pl.multiple_of(base + (c + s * per) * nrows, nrows)
        return src.at[pl.ds(r0, nrows)], dst.at[pl.ds(r0, nrows)]
    return f


def _issue_unit(f0, sem0, f1, sem1, c0=0, c1=PER):
    def body(c, carry):
        for s in range(NSUB):
            a, b = f0(c, s)
            pltpu.make_async_copy(a, b, sem0).start(priority=0)
            a, b = f1(c, s)
            pltpu.make_async_copy(a, b, sem1).start(priority=1)
        return carry
    jax.lax.fori_loop(c0, c1, body, 0)


def _wait_all(buf, sem):
    pltpu.make_async_copy(buf, buf, sem).wait()


def _make(R=3, CUTS=(0, 8, 16)):
    scale = DH ** -0.5
    NP = len(CUTS) - 1

    def kernel(x_hbm, g_hbm, k_hbm, v_hbm, wq_hbm, wo_hbm, c_hbm, wqb_hbm, wuk_hbm, wuv_hbm, wob_hbm,
               out_ref,
               kbuf, vbuf, wq_v, wo_v, c_v, wqb_v, wuk_v, wuv_v, wob_v, q_v, x_v, g_v, oa_v, cb_v, ksem, vsem, wsem, psem):
        def issue_kv(i, slot, c0=0, c1=PER):
            _issue_unit(_rows_chunk(k_hbm.at[i], kbuf.at[slot], 0, 128), ksem.at[slot],
                        _rows_chunk(v_hbm.at[i], vbuf.at[slot], 0, 128), vsem.at[slot], c0, c1)

        def wq_chunk(u):
            def f(c, s):
                r0 = pl.multiple_of(u * 256 + (c + PER * (s // 2)) * 8, 8)
                sl = (pl.ds(r0, 8), pl.ds((s % 2) * 2048, 2048))
                return wq_hbm.at[sl], wq_v.at[sl]
            return f

        def issue_wq_wuv(u):
            _issue_unit(wq_chunk(u), wsem.at[0], _rows_chunk(wuv_hbm, wuv_v, u * 8192, 128), wsem.at[8])

        def wo_chunk(src, dst, u):
            def f(c, s):
                r = pl.multiple_of(c * 32, 32)
                return src.at[pl.ds(pl.multiple_of(u * 2048 + s * 512 + r, 32), 32)], dst.at[4 * u + s, pl.ds(r, 32)]
            return f

        def issue_wo_wob(u):
            if u == 0:
                _issue_unit(wo_chunk(wo_hbm, wo_v, 0), wsem.at[1], wo_chunk(wob_hbm, wob_v, 0), wsem.at[9])
            else:
                for p in range(NP):
                    _issue_unit(wo_chunk(wo_hbm, wo_v, 1), psem.at[0, p], wo_chunk(wob_hbm, wob_v, 1), psem.at[1, p],
                                CUTS[p], CUTS[p + 1])

        def issue_wqb_wuk(u):
            _issue_unit(_rows_chunk(wqb_hbm, wqb_v, u * 8192, 128), wsem.at[2],
                        _rows_chunk(wuk_hbm, wuk_v, u * 8192, 128), wsem.at[3])

        def issue_c(qtr):
            _issue_unit(_rows_chunk(c_hbm.at[0], c_v.at[0], qtr * 2048, 32), wsem.at[4 + qtr // 2],
                        _rows_chunk(c_hbm.at[1], c_v.at[1], qtr * 2048, 32), wsem.at[6 + qtr // 2])

        cx = pltpu.make_async_copy(x_hbm, x_v, wsem.at[10])
        cg = pltpu.make_async_copy(g_hbm, g_v, wsem.at[11])
        cx.start()
        cg.start()
        issue_wqb_wuk(0)
        issue_wqb_wuk(1)
        issue_c(0)

        cx.wait()
        cg.wait()
        x2 = x_v[...]
        row16 = jax.lax.broadcasted_iota(jnp.int32, (ROWS, DM), 0)
        xf = x2.astype(jnp.float32)
        x16 = jnp.where(row16 == 0, xf[0:1, :], jnp.where(row16 == 1, xf[1:2, :], 0.0)).astype(jnp.bfloat16)
        rowbh = jax.lax.broadcasted_iota(jnp.int32, (NBH, DH), 0) % NH

        def qabs_pair(hp, qacc):
            wq0, wq1 = _pair_weights(wqb_v, hp)
            wk0, wk1 = _pair_weights(wuk_v, hp)
            for j, (wq_h, wk_h) in enumerate(((wq0, wk0), (wq1, wk1))):
                qh = jnp.dot(x16, wq_h, preferred_element_type=jnp.float32)
                qh = qh.astype(jnp.bfloat16).astype(jnp.float32)
                qb = jnp.concatenate([jnp.broadcast_to(qh[0:1, :], (NH, DH)),
                                      jnp.broadcast_to(qh[1:2, :], (NH, DH))], axis=0)
                lhs = jnp.where(rowbh == 2 * hp + j, qb, 0.0).astype(jnp.bfloat16)
                qacc = qacc + jax.lax.dot_general(lhs, wk_h, (((1,), (1,)), ((), ())),
                                                  preferred_element_type=jnp.float32)
            return qacc

        def b_half(b, hf, qabs):
            _wait_all(c_v.at[b, pl.ds(hf * HALF, HALF)], wsem.at[4 + 2 * b + hf])
            c = c_v[b, pl.ds(hf * HALF, HALF), :]
            s = jax.lax.dot_general(qabs[b * NH:(b + 1) * NH], c, (((1,), (1,)), ((), ())),
                                    preferred_element_type=jnp.float32) * scale
            m = jnp.max(s, axis=1, keepdims=True)
            p = jnp.exp(s - m)
            l = jnp.sum(p, axis=1, keepdims=True)
            cl = jnp.dot(p.astype(jnp.bfloat16), c, preferred_element_type=jnp.float32)
            return m, l, cl

        def merge(h0, h1):
            m0, l0, c0 = h0
            m1, l1, c1 = h1
            m = jnp.maximum(m0, m1)
            a0 = jnp.exp(m0 - m)
            a1 = jnp.exp(m1 - m)
            return (a0 * c0 + a1 * c1) / (a0 * l0 + a1 * l1)

        def ctx_pair(hp, ctxl):
            wv0, wv1 = _pair_weights(wuv_v, hp)
            for j, wv_h in enumerate((wv0, wv1)):
                h = 2 * hp + j
                lhs = jnp.where(row16 == 0, ctxl[h:h + 1, :],
                                jnp.where(row16 == 1, ctxl[NH + h:NH + h + 1, :], 0.0)).astype(jnp.bfloat16)
                r = jnp.dot(lhs, wv_h, preferred_element_type=jnp.float32)
                cb_v[:, h * DH:(h + 1) * DH] = r.astype(jnp.bfloat16)

        _wait_all(wqb_v, wsem.at[2])
        _wait_all(wuk_v, wsem.at[3])
        qabs = jnp.zeros((NBH, DC), jnp.float32)
        for hp in range(0, 4):
            qabs = qabs_pair(hp, qabs)
        issue_c(1)
        for hp in range(4, 8):
            qabs = qabs_pair(hp, qabs)
        issue_c(2)
        for hp in range(8, 12):
            qabs = qabs_pair(hp, qabs)
        issue_c(3)
        for hp in range(12, 16):
            qabs = qabs_pair(hp, qabs)
        qabs = qabs.astype(jnp.bfloat16)
        issue_wq_wuv(0)
        p00 = b_half(0, 0, qabs)
        issue_wq_wuv(1)
        p10 = b_half(1, 0, qabs)
        issue_kv(0, 0, 0, PER // 2)
        p01 = b_half(0, 1, qabs)
        issue_kv(0, 0, PER // 2, PER)
        p11 = b_half(1, 1, qabs)
        ctxl = jnp.concatenate([merge(p00, p01), merge(p10, p11)], axis=0)
        ctxl = ctxl.astype(jnp.bfloat16).astype(jnp.float32)
        issue_kv(1, 1, 0, PER // 2)
        _wait_all(wuv_v, wsem.at[8])
        _wait_all(wq_v, wsem.at[0])
        for hp in range(0, 8):
            ctx_pair(hp, ctxl)
        issue_kv(1, 1, PER // 2, PER)
        for hp in range(8, 16):
            ctx_pair(hp, ctxl)
        issue_kv(2, 2, 0, PER // 2)
        qa = jnp.dot(x16, wq_v[...], preferred_element_type=jnp.float32).astype(jnp.bfloat16)
        for h in range(NH):
            q_v[h] = qa[:, h * DH:(h + 1) * DH]
        gsum = jnp.sum(xf * g_v[...].reshape(1, DM).astype(jnp.float32), axis=1, keepdims=True)
        g = jax.nn.sigmoid(gsum)
        issue_kv(2, 2, PER // 2, PER)

        def head(i, carry):
            h = i % NH
            b = i // NH
            slot = i % R
            _wait_all(kbuf.at[slot], ksem.at[slot])
            s = jax.lax.dot_general(q_v[h], kbuf[slot], (((1,), (1,)), ((), ())),
                                    preferred_element_type=jnp.float32) * scale
            m = jnp.max(s, axis=1, keepdims=True)
            p = jnp.exp(s - m)
            l = jnp.sum(p, axis=1, keepdims=True)
            _wait_all(vbuf.at[slot], vsem.at[slot])
            o = jnp.dot(p.astype(jnp.bfloat16), vbuf[slot], preferred_element_type=jnp.float32)
            oa_v[b, :, pl.ds(pl.multiple_of(h * DH, DH), DH)] = (o / l).astype(jnp.bfloat16)

            @pl.when(i + R < NBH)
            def _():
                issue_kv(i + R, slot)

            @pl.when(i == NBH - R)
            def _():
                issue_wo_wob(0)

            @pl.when(i == NBH - R + 1)
            def _():
                issue_wo_wob(1)
            return carry

        jax.lax.fori_loop(0, NBH, head, 0)

        rowo = jax.lax.broadcasted_iota(jnp.int32, (ROWS, NH * DH), 0)
        oa = jnp.where(rowo == 0, oa_v[0], jnp.where(rowo == 1, oa_v[1], jnp.zeros((), jnp.bfloat16)))
        cb = cb_v[...]
        def proj(u, r0, nr, sem_a, sem_b):
            sl = (pl.ds(4 * u, 4), pl.ds(r0, nr))
            _wait_all(wo_v.at[sl], sem_a)
            _wait_all(wob_v.at[sl], sem_b)
            if nr == 512:
                la, lb = oa[:, 2048 * u:2048 * (u + 1)], cb[:, 2048 * u:2048 * (u + 1)]
            else:
                cols = [2048 * u + 512 * s_ + r0 for s_ in range(4)]
                la = jnp.concatenate([oa[:, c_:c_ + nr] for c_ in cols], axis=1)
                lb = jnp.concatenate([cb[:, c_:c_ + nr] for c_ in cols], axis=1)
            da = jnp.dot(la, wo_v[sl].reshape(4 * nr, DM), preferred_element_type=jnp.float32)
            db = jnp.dot(lb, wob_v[sl].reshape(4 * nr, DM), preferred_element_type=jnp.float32)
            return da, db

        acc_a, acc_b = proj(0, 0, 512, wsem.at[1], wsem.at[9])
        for p in range(NP):
            da, db = proj(1, CUTS[p] * 32, (CUTS[p + 1] - CUTS[p]) * 32, psem.at[0, p], psem.at[1, p])
            acc_a = acc_a + da
            acc_b = acc_b + db
        res = g * acc_a[0:2] + (1.0 - g) * acc_b[0:2]
        out_ref[...] = res.astype(out_ref.dtype)

    def run(A_x, A_k_cache, A_v_cache, A_wq, A_wo, B_x, B_c_kv, B_w_q, B_w_uk, B_w_uv, B_w_o, gate_w):
        del B_x
        x2 = A_x.reshape(NB, DM)
        k3 = A_k_cache.reshape(NBH, SK, DH)
        v3 = A_v_cache.reshape(NBH, SK, DH)
        wqb = B_w_q.reshape(DM * NH, DH)
        wuk = B_w_uk.reshape(DC * NH, DH)
        wuv = B_w_uv.reshape(DC * NH, DH)
        wob = B_w_o.reshape(NH * DH, DM)
        any_spec = pl.BlockSpec(memory_space=pl.ANY)
        vm = pl.BlockSpec(memory_space=pltpu.VMEM)
        bf = jnp.bfloat16
        out = pl.pallas_call(
            kernel,
            in_specs=[any_spec] * 11,
            out_specs=vm,
            out_shape=jax.ShapeDtypeStruct((NB, DM), bf),
            scratch_shapes=[
                pltpu.VMEM((R, SK, DH), bf), pltpu.VMEM((R, SK, DH), bf),
                pltpu.VMEM((DM, NH * DH), bf), pltpu.VMEM((8, 512, DM), bf),
                pltpu.VMEM((NB, SK, DC), bf),
                pltpu.VMEM((DM * NH, DH), bf), pltpu.VMEM((DC * NH, DH), bf), pltpu.VMEM((DC * NH, DH), bf),
                pltpu.VMEM((8, 512, DM), bf),
                pltpu.VMEM((NH, ROWS, DH), bf),
                pltpu.VMEM((NB, DM), bf), pltpu.VMEM((DM,), bf),
                pltpu.VMEM((NB, ROWS, NH * DH), bf), pltpu.VMEM((ROWS, NH * DH), bf),
                pltpu.SemaphoreType.DMA((R,)), pltpu.SemaphoreType.DMA((R,)), pltpu.SemaphoreType.DMA((12,)), pltpu.SemaphoreType.DMA((2, NP)),
            ],
            compiler_params=pltpu.CompilerParams(vmem_limit_bytes=110 * 1024 * 1024),
        )(x2, gate_w, k3, v3, A_wq, A_wo, B_c_kv, wqb, wuk, wuv, wob)
        return out.reshape(NB, 1, DM)

    return run


@jax.jit
def pallas_gated_mix__mha_block_cached__compressed_kv_cla__decode_kernel(
    A_x, A_k_cache, A_v_cache, A_wq, A_wo, B_x, B_c_kv, B_w_q, B_w_uk, B_w_uv, B_w_o, gate_w,
):
    return _make()(A_x, A_k_cache, A_v_cache, A_wq, A_wo, B_x, B_c_kv, B_w_q, B_w_uk, B_w_uv, B_w_o, gate_w)
```

```python
import jax
import jax.numpy as jnp
import jax.experimental.pallas as pl
import jax.experimental.pallas.tpu as pltpu

NB, NH, SK, DH, DM, DC = 2, 32, 8192, 128, 512, 512
NBH = NB * NH
ROWS = 16
HALF = SK // 2
CBLK = DH * NH
NSUB = 4
PER = 16
RING = 3
LAST_CUT = PER // 2
SCALE = DH ** -0.5

S_WQ, S_WO, S_WQB, S_WUK, S_C, S_WUV, S_WOB, S_X, S_G = 0, 1, 2, 3, 4, 8, 9, 10, 11
N_WSEM = 12

_NT = (((1,), (1,)), ((), ()))


def _issue(chunk0, sem0, chunk1, sem1, c0=0, c1=PER):
    def body(c, carry):
        for s in range(NSUB):
            pltpu.make_async_copy(*chunk0(c, s), sem0).start(priority=0)
            pltpu.make_async_copy(*chunk1(c, s), sem1).start(priority=1)
        return carry
    jax.lax.fori_loop(c0, c1, body, 0)


def _wait_all(buf, sem):
    pltpu.make_async_copy(buf, buf, sem).wait()


def _row_chunks(src, dst, base, nrows):
    def chunk(c, s):
        rows = pl.ds(pl.multiple_of(base + (c + s * PER) * nrows, nrows), nrows)
        return src.at[rows], dst.at[rows]
    return chunk


def _dot(a, b):
    return jnp.dot(a, b, preferred_element_type=jnp.float32)


def _dot_nt(a, b):
    return jax.lax.dot_general(a, b, _NT, preferred_element_type=jnp.float32)


def _kernel(x_hbm, g_hbm, k_hbm, v_hbm, wq_hbm, wo_hbm, c_hbm, wqb_hbm, wuk_hbm, wuv_hbm, wob_hbm,
            out_ref,
            kbuf, vbuf, wq_v, wo_v, c_v, wqb_v, wuk_v, wuv_v, wob_v, x_v, g_v, q_v, oa_v, cb_v, e0_v,
            ksem, vsem, wsem, psem):
    bf16 = jnp.bfloat16

    def issue_kv(i, slot, c0=0, c1=PER):
        _issue(_row_chunks(k_hbm.at[i], kbuf.at[slot], 0, 128), ksem.at[slot],
               _row_chunks(v_hbm.at[i], vbuf.at[slot], 0, 128), vsem.at[slot], c0, c1)

    def issue_wqb_wuk(u):
        _issue(_row_chunks(wqb_hbm, wqb_v, u * 8192, 128), wsem.at[S_WQB],
               _row_chunks(wuk_hbm, wuk_v, u * 8192, 128), wsem.at[S_WUK])

    def issue_c(qtr):
        _issue(_row_chunks(c_hbm.at[0], c_v.at[0], qtr * 2048, 32), wsem.at[S_C + qtr // 2],
               _row_chunks(c_hbm.at[1], c_v.at[1], qtr * 2048, 32), wsem.at[S_C + 2 + qtr // 2])

    def issue_wq_wuv(u):
        def wq_chunk(c, s):
            sl = (pl.ds(pl.multiple_of(u * 256 + (c + PER * (s // 2)) * 8, 8), 8), pl.ds((s % 2) * 2048, 2048))
            return wq_hbm.at[sl], wq_v.at[sl]
        _issue(wq_chunk, wsem.at[S_WQ], _row_chunks(wuv_hbm, wuv_v, u * 8192, 128), wsem.at[S_WUV])

    def wo_chunks(src, dst, u):
        def chunk(c, s):
            r = pl.multiple_of(c * 32, 32)
            return src.at[pl.ds(pl.multiple_of(u * 2048 + s * 512 + r, 32), 32)], dst.at[4 * u + s, pl.ds(r, 32)]
        return chunk

    def issue_wo_wob(u):
        if u == 0:
            _issue(wo_chunks(wo_hbm, wo_v, 0), wsem.at[S_WO], wo_chunks(wob_hbm, wob_v, 0), wsem.at[S_WOB])
        else:
            for p, (c0, c1) in enumerate(((0, LAST_CUT), (LAST_CUT, PER))):
                _issue(wo_chunks(wo_hbm, wo_v, 1), psem.at[0, p], wo_chunks(wob_hbm, wob_v, 1), psem.at[1, p], c0, c1)

    cx = pltpu.make_async_copy(x_hbm, x_v, wsem.at[S_X])
    cg = pltpu.make_async_copy(g_hbm, g_v, wsem.at[S_G])
    cx.start()
    cg.start()
    issue_wqb_wuk(0)
    e0_v[...] = (jax.lax.broadcasted_iota(jnp.int32, (DH, CBLK), 1) // NH
                 == jax.lax.broadcasted_iota(jnp.int32, (DH, CBLK), 0)).astype(bf16)
    issue_wqb_wuk(1)
    issue_c(0)

    cx.wait()
    cg.wait()
    row16 = jax.lax.broadcasted_iota(jnp.int32, (ROWS, DM), 0)
    xf = x_v[...].astype(jnp.float32)
    x16 = jnp.where(row16 == 0, xf[0:1, :], jnp.where(row16 == 1, xf[1:2, :], 0.0)).astype(bf16)

    E0 = e0_v[...]
    diag = (jax.lax.broadcasted_iota(jnp.int32, (NBH, CBLK), 0) % NH
            == jax.lax.broadcasted_iota(jnp.int32, (NBH, CBLK), 1) % NH)

    def q_block(j, acc):
        xr = _dot(x16[:, j * DH:(j + 1) * DH], E0)
        xb = jnp.concatenate([jnp.broadcast_to(xr[0:1, :], (NH, CBLK)),
                              jnp.broadcast_to(xr[1:2, :], (NH, CBLK))], axis=0)
        lhs = jnp.where(diag, xb, 0.0).astype(bf16)
        return acc + _dot(lhs, wqb_v[pl.ds(j * CBLK, CBLK), :])

    def qabs_block(j, q64):
        r = _dot_nt(q64, wuk_v[pl.ds(j * CBLK, CBLK), :])
        return _dot_nt(jnp.where(diag, r, 0.0).astype(bf16), E0)

    def latent_attention_half(b, hf, qabs):
        rows = pl.ds(hf * HALF, HALF)
        _wait_all(c_v.at[b, rows], wsem.at[S_C + 2 * b + hf])
        c = c_v[b, rows, :]
        s = _dot_nt(qabs[b * NH:(b + 1) * NH], c) * SCALE
        m = jnp.max(s, axis=1, keepdims=True)
        p = jnp.exp(s - m)
        return m, jnp.sum(p, axis=1, keepdims=True), _dot(p.astype(bf16), c)

    def merge(h0, h1):
        (m0, l0, c0), (m1, l1, c1) = h0, h1
        m = jnp.maximum(m0, m1)
        a0, a1 = jnp.exp(m0 - m), jnp.exp(m1 - m)
        return (a0 * c0 + a1 * c1) / (a0 * l0 + a1 * l1)

    def ctx_block(j, ctxl, acc):
        e = _dot(ctxl[:, j * DH:(j + 1) * DH], E0)
        lhs = jnp.where(diag, e, 0.0).astype(bf16)
        return acc + _dot(lhs, wuv_v[pl.ds(j * CBLK, CBLK), :])

    _wait_all(wqb_v, wsem.at[S_WQB])
    _wait_all(wuk_v, wsem.at[S_WUK])
    q64 = jnp.zeros((NBH, DH), jnp.float32)
    for j in range(4):
        q64 = q_block(j, q64)
    q64 = q64.astype(bf16)
    issue_c(1)
    qparts = [qabs_block(0, q64), qabs_block(1, q64)]
    issue_c(2)
    qparts += [qabs_block(2, q64), qabs_block(3, q64)]
    qabs = jnp.concatenate(qparts, axis=1).astype(bf16)
    issue_c(3)
    p00 = latent_attention_half(0, 0, qabs)
    issue_wq_wuv(0)
    p10 = latent_attention_half(1, 0, qabs)
    issue_wq_wuv(1)
    p01 = latent_attention_half(0, 1, qabs)
    issue_kv(0, 0, 0, PER // 2)
    p11 = latent_attention_half(1, 1, qabs)
    ctxl = jnp.concatenate([merge(p00, p01), merge(p10, p11)], axis=0).astype(bf16)
    issue_kv(0, 0, PER // 2, PER)
    _wait_all(wuv_v, wsem.at[S_WUV])
    _wait_all(wq_v, wsem.at[S_WQ])
    ctx = jnp.zeros((NBH, DH), jnp.float32)
    for j in range(2):
        ctx = ctx_block(j, ctxl, ctx)
    issue_kv(1, 1, 0, PER // 2)
    for j in range(2, 4):
        ctx = ctx_block(j, ctxl, ctx)
    rowh = jax.lax.broadcasted_iota(jnp.int32, (ROWS, DH), 0)
    for h in range(NH):
        cb_v[:, h * DH:(h + 1) * DH] = jnp.where(
            rowh == 0, ctx[h:h + 1, :], jnp.where(rowh == 1, ctx[NH + h:NH + h + 1, :], 0.0)).astype(bf16)
    issue_kv(1, 1, PER // 2, PER)
    qa = _dot(x16, wq_v[...]).astype(bf16)
    for h in range(NH):
        q_v[h] = qa[:, h * DH:(h + 1) * DH]
    g = jax.nn.sigmoid(jnp.sum(xf * g_v[...].reshape(1, DM).astype(jnp.float32), axis=1, keepdims=True))
    issue_kv(2, 2)

    def head(i, carry):
        h = i % NH
        b = i // NH
        slot = i % RING
        _wait_all(kbuf.at[slot], ksem.at[slot])
        s = _dot_nt(q_v[h], kbuf[slot]) * SCALE
        m = jnp.max(s, axis=1, keepdims=True)
        p = jnp.exp(s - m)
        l = jnp.sum(p, axis=1, keepdims=True)
        _wait_all(vbuf.at[slot], vsem.at[slot])
        o = _dot(p.astype(bf16), vbuf[slot])
        oa_v[b, :, pl.ds(pl.multiple_of(h * DH, DH), DH)] = (o / l).astype(bf16)

        @pl.when(i + RING < NBH)
        def _():
            issue_kv(i + RING, slot)

        @pl.when(i == NBH - RING)
        def _():
            issue_wo_wob(0)

        @pl.when(i == NBH - RING + 1)
        def _():
            issue_wo_wob(1)
        return carry

    jax.lax.fori_loop(0, NBH, head, 0)

    rowo = jax.lax.broadcasted_iota(jnp.int32, (ROWS, NH * DH), 0)
    oa = jnp.where(rowo == 0, oa_v[0], jnp.where(rowo == 1, oa_v[1], jnp.zeros((), bf16)))
    cb = cb_v[...]

    def project(u, r0, nr, sem_a, sem_b):
        sl = (pl.ds(4 * u, 4), pl.ds(r0, nr))
        _wait_all(wo_v.at[sl], sem_a)
        _wait_all(wob_v.at[sl], sem_b)
        cols = [2048 * u + 512 * s + r0 for s in range(4)]
        la = jnp.concatenate([oa[:, c0:c0 + nr] for c0 in cols], axis=1)
        lb = jnp.concatenate([cb[:, c0:c0 + nr] for c0 in cols], axis=1)
        return _dot(la, wo_v[sl].reshape(4 * nr, DM)), _dot(lb, wob_v[sl].reshape(4 * nr, DM))

    acc_a, acc_b = project(0, 0, 512, wsem.at[S_WO], wsem.at[S_WOB])
    for p, (c0, c1) in enumerate(((0, LAST_CUT), (LAST_CUT, PER))):
        da, db = project(1, c0 * 32, (c1 - c0) * 32, psem.at[0, p], psem.at[1, p])
        acc_a, acc_b = acc_a + da, acc_b + db
    out_ref[...] = (g * acc_a[0:NB] + (1.0 - g) * acc_b[0:NB]).astype(out_ref.dtype)


@jax.jit
def pallas_gated_mix__mha_block_cached__compressed_kv_cla__decode_kernel(
    A_x: jax.Array,
    A_k_cache: jax.Array,
    A_v_cache: jax.Array,
    A_wq: jax.Array,
    A_wo: jax.Array,
    B_x: jax.Array,
    B_c_kv: jax.Array,
    B_w_q: jax.Array,
    B_w_uk: jax.Array,
    B_w_uv: jax.Array,
    B_w_o: jax.Array,
    gate_w: jax.Array,
):
    del B_x
    bf = jnp.bfloat16
    hbm = pl.BlockSpec(memory_space=pl.ANY)
    out = pl.pallas_call(
        _kernel,
        in_specs=[hbm] * 11,
        out_specs=pl.BlockSpec(memory_space=pltpu.VMEM),
        out_shape=jax.ShapeDtypeStruct((NB, DM), bf),
        scratch_shapes=[
            pltpu.VMEM((RING, SK, DH), bf),
            pltpu.VMEM((RING, SK, DH), bf),
            pltpu.VMEM((DM, NH * DH), bf),
            pltpu.VMEM((8, 512, DM), bf),
            pltpu.VMEM((NB, SK, DC), bf),
            pltpu.VMEM((DM * NH, DH), bf),
            pltpu.VMEM((DC * NH, DH), bf),
            pltpu.VMEM((DC * NH, DH), bf),
            pltpu.VMEM((8, 512, DM), bf),
            pltpu.VMEM((NB, DM), bf),
            pltpu.VMEM((DM,), bf),
            pltpu.VMEM((NH, ROWS, DH), bf),
            pltpu.VMEM((NB, ROWS, NH * DH), bf),
            pltpu.VMEM((ROWS, NH * DH), bf),
            pltpu.VMEM((DH, CBLK), bf),
            pltpu.SemaphoreType.DMA((RING,)),
            pltpu.SemaphoreType.DMA((RING,)),
            pltpu.SemaphoreType.DMA((N_WSEM,)),
            pltpu.SemaphoreType.DMA((2, 2)),
        ],
        compiler_params=pltpu.CompilerParams(vmem_limit_bytes=100 * 1024 * 1024),
    )(
        A_x.reshape(NB, DM),
        gate_w,
        A_k_cache.reshape(NBH, SK, DH),
        A_v_cache.reshape(NBH, SK, DH),
        A_wq,
        A_wo,
        B_c_kv,
        B_w_q.reshape(DM * NH, DH),
        B_w_uk.reshape(DC * NH, DH),
        B_w_uv.reshape(DC * NH, DH),
        B_w_o.reshape(NH * DH, DM),
    )
    return out.reshape(NB, 1, DM)
```

```python
import jax
import jax.numpy as jnp
import jax.experimental.pallas as pl
import jax.experimental.pallas.tpu as pltpu

NB, NH, SK, DH, DM, DC = 2, 32, 8192, 128, 512, 512
NBH = NB * NH
ROWS = 16
HALF = SK // 2
CBLK = DH * NH
NSUB = 4
PER = 16
RING = 3
LAST_CUT = 12
SCALE = DH ** -0.5

S_WQ, S_WO, S_WQB, S_WUK, S_C, S_WUV, S_WOB, S_X, S_G = 0, 1, 2, 3, 4, 8, 9, 10, 11
N_WSEM = 12

_NT = (((1,), (1,)), ((), ()))


def _issue(chunk0, sem0, chunk1, sem1, c0=0, c1=PER):
    def body(c, carry):
        for s in range(NSUB):
            pltpu.make_async_copy(*chunk0(c, s), sem0).start(priority=0)
            pltpu.make_async_copy(*chunk1(c, s), sem1).start(priority=1)
        return carry
    jax.lax.fori_loop(c0, c1, body, 0)


def _wait_all(buf, sem):
    pltpu.make_async_copy(buf, buf, sem).wait()


def _row_chunks(src, dst, base, nrows):
    def chunk(c, s):
        rows = pl.ds(pl.multiple_of(base + (c + s * PER) * nrows, nrows), nrows)
        return src.at[rows], dst.at[rows]
    return chunk


def _dot(a, b):
    return jnp.dot(a, b, preferred_element_type=jnp.float32)


def _dot_nt(a, b):
    return jax.lax.dot_general(a, b, _NT, preferred_element_type=jnp.float32)


def _kernel(x_hbm, g_hbm, k_hbm, v_hbm, wq_hbm, wo_hbm, c_hbm, wqb_hbm, wuk_hbm, wuv_hbm, wob_hbm,
            out_ref,
            kbuf, vbuf, wq_v, wo_v, c_v, wqb_v, wuk_v, wuv_v, wob_v, x_v, g_v, q_v, oa_v, cb_v, e0_v, acc_v,
            ksem, vsem, wsem, psem):
    bf16 = jnp.bfloat16

    def issue_kv(i, slot, c0=0, c1=PER):
        _issue(_row_chunks(k_hbm.at[i], kbuf.at[slot], 0, 128), ksem.at[slot],
               _row_chunks(v_hbm.at[i], vbuf.at[slot], 0, 128), vsem.at[slot], c0, c1)

    def issue_wqb_wuk(u):
        _issue(_row_chunks(wqb_hbm, wqb_v, u * 8192, 128), wsem.at[S_WQB],
               _row_chunks(wuk_hbm, wuk_v, u * 8192, 128), wsem.at[S_WUK])

    def issue_c(qtr):
        _issue(_row_chunks(c_hbm.at[0], c_v.at[0], qtr * 2048, 32), wsem.at[S_C + qtr // 2],
               _row_chunks(c_hbm.at[1], c_v.at[1], qtr * 2048, 32), wsem.at[S_C + 2 + qtr // 2])

    def issue_wq_wuv(u):
        def wq_chunk(c, s):
            sl = (pl.ds(pl.multiple_of(u * 256 + (c + PER * (s // 2)) * 8, 8), 8), pl.ds((s % 2) * 2048, 2048))
            return wq_hbm.at[sl], wq_v.at[sl]
        _issue(wq_chunk, wsem.at[S_WQ], _row_chunks(wuv_hbm, wuv_v, u * 8192, 128), wsem.at[S_WUV])

    def wo_chunks(src, dst, u):
        def chunk(c, s):
            r = pl.multiple_of(c * 32, 32)
            return src.at[pl.ds(pl.multiple_of(u * 2048 + s * 512 + r, 32), 32)], dst.at[4 * u + s, pl.ds(r, 32)]
        return chunk

    def issue_wo_wob0():
        _issue(wo_chunks(wo_hbm, wo_v, 0), wsem.at[S_WO], wo_chunks(wob_hbm, wob_v, 0), wsem.at[S_WOB])

    cx = pltpu.make_async_copy(x_hbm, x_v, wsem.at[S_X])
    cg = pltpu.make_async_copy(g_hbm, g_v, wsem.at[S_G])
    cx.start()
    cg.start()
    issue_wqb_wuk(0)
    e0_v[...] = (jax.lax.broadcasted_iota(jnp.int32, (DH, CBLK), 1) // NH
                 == jax.lax.broadcasted_iota(jnp.int32, (DH, CBLK), 0)).astype(bf16)
    issue_wqb_wuk(1)
    issue_c(0)

    cx.wait()
    cg.wait()
    row16 = jax.lax.broadcasted_iota(jnp.int32, (ROWS, DM), 0)
    xf = x_v[...].astype(jnp.float32)
    x16 = jnp.where(row16 == 0, xf[0:1, :], jnp.where(row16 == 1, xf[1:2, :], 0.0)).astype(bf16)

    E0 = e0_v[...]
    diag = (jax.lax.broadcasted_iota(jnp.int32, (NBH, CBLK), 0) % NH
            == jax.lax.broadcasted_iota(jnp.int32, (NBH, CBLK), 1) % NH)

    def q_block(j, acc):
        xr = _dot(x16[:, j * DH:(j + 1) * DH], E0)
        xb = jnp.concatenate([jnp.broadcast_to(xr[0:1, :], (NH, CBLK)),
                              jnp.broadcast_to(xr[1:2, :], (NH, CBLK))], axis=0)
        lhs = jnp.where(diag, xb, 0.0).astype(bf16)
        return acc + _dot(lhs, wqb_v[pl.ds(j * CBLK, CBLK), :])

    def qabs_block(j, q64):
        r = _dot_nt(q64, wuk_v[pl.ds(j * CBLK, CBLK), :])
        return _dot_nt(jnp.where(diag, r, 0.0).astype(bf16), E0)

    def latent_attention_half(b, hf, qabs):
        rows = pl.ds(hf * HALF, HALF)
        _wait_all(c_v.at[b, rows], wsem.at[S_C + 2 * b + hf])
        c = c_v[b, rows, :]
        s = _dot_nt(qabs[b * NH:(b + 1) * NH], c) * SCALE
        m = jnp.max(s, axis=1, keepdims=True)
        p = jnp.exp(s - m)
        return m, jnp.sum(p, axis=1, keepdims=True), _dot(p.astype(bf16), c)

    def merge(h0, h1):
        (m0, l0, c0), (m1, l1, c1) = h0, h1
        m = jnp.maximum(m0, m1)
        a0, a1 = jnp.exp(m0 - m), jnp.exp(m1 - m)
        return (a0 * c0 + a1 * c1) / (a0 * l0 + a1 * l1)

    def ctx_block(j, ctxl, acc):
        e = _dot(ctxl[:, j * DH:(j + 1) * DH], E0)
        lhs = jnp.where(diag, e, 0.0).astype(bf16)
        return acc + _dot(lhs, wuv_v[pl.ds(j * CBLK, CBLK), :])

    _wait_all(wqb_v, wsem.at[S_WQB])
    _wait_all(wuk_v, wsem.at[S_WUK])
    q64 = jnp.zeros((NBH, DH), jnp.float32)
    for j in range(4):
        q64 = q_block(j, q64)
    q64 = q64.astype(bf16)
    issue_c(1)
    qparts = [qabs_block(0, q64), qabs_block(1, q64)]
    issue_c(2)
    qparts += [qabs_block(2, q64), qabs_block(3, q64)]
    qabs = jnp.concatenate(qparts, axis=1).astype(bf16)
    issue_c(3)
    p00 = latent_attention_half(0, 0, qabs)
    issue_wq_wuv(0)
    p10 = latent_attention_half(1, 0, qabs)
    issue_wq_wuv(1)
    p01 = latent_attention_half(0, 1, qabs)
    issue_kv(0, 0, 0, PER // 2)
    p11 = latent_attention_half(1, 1, qabs)
    ctxl = jnp.concatenate([merge(p00, p01), merge(p10, p11)], axis=0).astype(bf16)
    issue_kv(0, 0, PER // 2, PER)
    _wait_all(wuv_v, wsem.at[S_WUV])
    _wait_all(wq_v, wsem.at[S_WQ])
    ctx = jnp.zeros((NBH, DH), jnp.float32)
    for j in range(2):
        ctx = ctx_block(j, ctxl, ctx)
    issue_kv(1, 1, 0, PER // 2)
    for j in range(2, 4):
        ctx = ctx_block(j, ctxl, ctx)
    rowh = jax.lax.broadcasted_iota(jnp.int32, (ROWS, DH), 0)
    for h in range(NH):
        cb_v[:, h * DH:(h + 1) * DH] = jnp.where(
            rowh == 0, ctx[h:h + 1, :], jnp.where(rowh == 1, ctx[NH + h:NH + h + 1, :], 0.0)).astype(bf16)
    issue_kv(1, 1, PER // 2, PER)
    qa = _dot(x16, wq_v[...]).astype(bf16)
    for h in range(NH):
        q_v[h] = qa[:, h * DH:(h + 1) * DH]
    g = jax.nn.sigmoid(jnp.sum(xf * g_v[...].reshape(1, DM).astype(jnp.float32), axis=1, keepdims=True))
    issue_kv(2, 2)

    def project(u, r0, nr, sem_a, sem_b):
        sl = (pl.ds(4 * u, 4), pl.ds(r0, nr))
        _wait_all(wo_v.at[sl], sem_a)
        _wait_all(wob_v.at[sl], sem_b)
        cols = [pl.ds(2048 * u + 512 * s + r0, nr) for s in range(4)]
        rowp = jax.lax.broadcasted_iota(jnp.int32, (ROWS, 4 * nr), 0)
        la = jnp.where(rowp == 0, jnp.concatenate([oa_v[0, :, c] for c in cols], axis=1),
                       jnp.where(rowp == 1, jnp.concatenate([oa_v[1, :, c] for c in cols], axis=1),
                                 jnp.zeros((), bf16)))
        lb = jnp.concatenate([cb_v[:, c] for c in cols], axis=1)
        return _dot(la, wo_v[sl].reshape(4 * nr, DM)), _dot(lb, wob_v[sl].reshape(4 * nr, DM))

    def head(i, carry):
        h = i % NH
        b = i // NH
        slot = i % RING
        _wait_all(kbuf.at[slot], ksem.at[slot])
        s = _dot_nt(q_v[h], kbuf[slot]) * SCALE
        m = jnp.max(s, axis=1, keepdims=True)
        p = jnp.exp(s - m)
        l = jnp.sum(p, axis=1, keepdims=True)
        _wait_all(vbuf.at[slot], vsem.at[slot])
        o = _dot(p.astype(bf16), vbuf[slot])
        oa_v[b, :, pl.ds(pl.multiple_of(h * DH, DH), DH)] = (o / l).astype(bf16)

        @pl.when(i + RING < NBH)
        def _():
            issue_kv(i + RING, slot)

        @pl.when(i == NBH - RING)
        def _():
            issue_wo_wob0()

        @pl.when(i == NBH - RING + 1)
        def _():
            _issue(wo_chunks(wo_hbm, wo_v, 1), psem.at[0, 0], wo_chunks(wob_hbm, wob_v, 1), psem.at[1, 0], 0, LAST_CUT)
            acc_v[0], acc_v[1] = project(0, 0, 512, wsem.at[S_WO], wsem.at[S_WOB])
            _issue(wo_chunks(wo_hbm, wo_v, 1), psem.at[0, 1], wo_chunks(wob_hbm, wob_v, 1), psem.at[1, 1], LAST_CUT, PER)
        return carry

    jax.lax.fori_loop(0, NBH, head, 0)

    acc_a, acc_b = acc_v[0], acc_v[1]
    for p, (c0, c1) in enumerate(((0, LAST_CUT), (LAST_CUT, PER))):
        da, db = project(1, c0 * 32, (c1 - c0) * 32, psem.at[0, p], psem.at[1, p])
        acc_a, acc_b = acc_a + da, acc_b + db
    out_ref[...] = (g * acc_a[0:NB] + (1.0 - g) * acc_b[0:NB]).astype(out_ref.dtype)


@jax.jit
def pallas_gated_mix__mha_block_cached__compressed_kv_cla__decode_kernel(
    A_x: jax.Array,
    A_k_cache: jax.Array,
    A_v_cache: jax.Array,
    A_wq: jax.Array,
    A_wo: jax.Array,
    B_x: jax.Array,
    B_c_kv: jax.Array,
    B_w_q: jax.Array,
    B_w_uk: jax.Array,
    B_w_uv: jax.Array,
    B_w_o: jax.Array,
    gate_w: jax.Array,
):
    del B_x
    bf = jnp.bfloat16
    hbm = pl.BlockSpec(memory_space=pl.ANY)
    out = pl.pallas_call(
        _kernel,
        in_specs=[hbm] * 11,
        out_specs=pl.BlockSpec(memory_space=pltpu.VMEM),
        out_shape=jax.ShapeDtypeStruct((NB, DM), bf),
        scratch_shapes=[
            pltpu.VMEM((RING, SK, DH), bf),
            pltpu.VMEM((RING, SK, DH), bf),
            pltpu.VMEM((DM, NH * DH), bf),
            pltpu.VMEM((8, 512, DM), bf),
            pltpu.VMEM((NB, SK, DC), bf),
            pltpu.VMEM((DM * NH, DH), bf),
            pltpu.VMEM((DC * NH, DH), bf),
            pltpu.VMEM((DC * NH, DH), bf),
            pltpu.VMEM((8, 512, DM), bf),
            pltpu.VMEM((NB, DM), bf),
            pltpu.VMEM((DM,), bf),
            pltpu.VMEM((NH, ROWS, DH), bf),
            pltpu.VMEM((NB, ROWS, NH * DH), bf),
            pltpu.VMEM((ROWS, NH * DH), bf),
            pltpu.VMEM((DH, CBLK), bf),
            pltpu.VMEM((2, ROWS, DM), jnp.float32),
            pltpu.SemaphoreType.DMA((RING,)),
            pltpu.SemaphoreType.DMA((RING,)),
            pltpu.SemaphoreType.DMA((N_WSEM,)),
            pltpu.SemaphoreType.DMA((2, 2)),
        ],
        compiler_params=pltpu.CompilerParams(vmem_limit_bytes=100 * 1024 * 1024),
    )(
        A_x.reshape(NB, DM),
        gate_w,
        A_k_cache.reshape(NBH, SK, DH),
        A_v_cache.reshape(NBH, SK, DH),
        A_wq,
        A_wo,
        B_c_kv,
        B_w_q.reshape(DM * NH, DH),
        B_w_uk.reshape(DC * NH, DH),
        B_w_uv.reshape(DC * NH, DH),
        B_w_o.reshape(NH * DH, DM),
    )
    return out.reshape(NB, 1, DM)
```

```python
import jax
import jax.numpy as jnp
import jax.experimental.pallas as pl
import jax.experimental.pallas.tpu as pltpu

NB, NH, SK, DH, DM, DC = 2, 32, 8192, 128, 512, 512
NBH = NB * NH
ROWS = 16
HALF = SK // 2
CBLK = DH * NH
NSUB = 4
PER = 16
RING = 3
LAST_CUT = 12
SCALE = DH ** -0.5
assert RING == 3 and NSUB * PER * 128 == SK

S_WQ, S_WO, S_WQB, S_WUK, S_C, S_WUV, S_WOB, S_X, S_G = 0, 1, 2, 3, 4, 8, 9, 10, 11
N_WSEM = 12

_NT = (((1,), (1,)), ((), ()))


def _issue(chunk0, sem0, chunk1, sem1, c0=0, c1=PER):
    def body(c, carry):
        for s in range(NSUB):
            pltpu.make_async_copy(*chunk0(c, s), sem0).start(priority=0)
            pltpu.make_async_copy(*chunk1(c, s), sem1).start(priority=1)
        return carry
    jax.lax.fori_loop(c0, c1, body, 0)


def _wait_all(buf, sem):
    pltpu.make_async_copy(buf, buf, sem).wait()


def _row_chunks(src, dst, base, nrows):
    def chunk(c, s):
        rows = pl.ds(pl.multiple_of(base + (c + s * PER) * nrows, nrows), nrows)
        return src.at[rows], dst.at[rows]
    return chunk


def _dot(a, b):
    return jnp.dot(a, b, preferred_element_type=jnp.float32)


def _dot_nt(a, b):
    return jax.lax.dot_general(a, b, _NT, preferred_element_type=jnp.float32)


def _kernel(x_hbm, g_hbm, k_hbm, v_hbm, wq_hbm, wo_hbm, c_hbm, wqb_hbm, wuk_hbm, wuv_hbm, wob_hbm,
            out_ref,
            kbuf, vbuf, wq_v, wo_v, c_v, wqb_v, wuk_v, wuv_v, wob_v, x_v, g_v, q_v, oa_v, cb_v, e0_v, acc_v,
            ksem, vsem, wsem, psem):
    bf16 = jnp.bfloat16

    def issue_kv(i, slot, c0=0, c1=PER):
        _issue(_row_chunks(k_hbm.at[i], kbuf.at[slot], 0, 128), ksem.at[slot],
               _row_chunks(v_hbm.at[i], vbuf.at[slot], 0, 128), vsem.at[slot], c0, c1)

    def issue_wqb_wuk(u):
        _issue(_row_chunks(wqb_hbm, wqb_v, u * 8192, 128), wsem.at[S_WQB],
               _row_chunks(wuk_hbm, wuk_v, u * 8192, 128), wsem.at[S_WUK])

    def issue_c(qtr):
        _issue(_row_chunks(c_hbm.at[0], c_v.at[0], qtr * 2048, 32), wsem.at[S_C + qtr // 2],
               _row_chunks(c_hbm.at[1], c_v.at[1], qtr * 2048, 32), wsem.at[S_C + 2 + qtr // 2])

    def issue_wq_wuv(u):
        def wq_chunk(c, s):
            sl = (pl.ds(pl.multiple_of(u * 256 + (c + PER * (s // 2)) * 8, 8), 8), pl.ds((s % 2) * 2048, 2048))
            return wq_hbm.at[sl], wq_v.at[sl]
        _issue(wq_chunk, wsem.at[S_WQ], _row_chunks(wuv_hbm, wuv_v, u * 8192, 128), wsem.at[S_WUV])

    def wo_chunks(src, dst, u):
        def chunk(c, s):
            r = pl.multiple_of(c * 32, 32)
            return src.at[pl.ds(pl.multiple_of(u * 2048 + s * 512 + r, 32), 32)], dst.at[4 * u + s, pl.ds(r, 32)]
        return chunk

    def issue_wo_wob0():
        _issue(wo_chunks(wo_hbm, wo_v, 0), wsem.at[S_WO], wo_chunks(wob_hbm, wob_v, 0), wsem.at[S_WOB])

    cx = pltpu.make_async_copy(x_hbm, x_v, wsem.at[S_X])
    cg = pltpu.make_async_copy(g_hbm, g_v, wsem.at[S_G])
    cx.start()
    cg.start()
    issue_wqb_wuk(0)
    e0_v[...] = (jax.lax.broadcasted_iota(jnp.int32, (DH, CBLK), 1) // NH
                 == jax.lax.broadcasted_iota(jnp.int32, (DH, CBLK), 0)).astype(bf16)
    issue_wqb_wuk(1)
    issue_c(0)

    cx.wait()
    cg.wait()
    row16 = jax.lax.broadcasted_iota(jnp.int32, (ROWS, DM), 0)
    xf = x_v[...].astype(jnp.float32)
    x16 = jnp.where(row16 == 0, xf[0:1, :], jnp.where(row16 == 1, xf[1:2, :], 0.0)).astype(bf16)

    E0 = e0_v[...]
    diag = (jax.lax.broadcasted_iota(jnp.int32, (NBH, CBLK), 0) % NH
            == jax.lax.broadcasted_iota(jnp.int32, (NBH, CBLK), 1) % NH)

    def q_block(j, acc):
        xr = _dot(x16[:, j * DH:(j + 1) * DH], E0)
        xb = jnp.concatenate([jnp.broadcast_to(xr[0:1, :], (NH, CBLK)),
                              jnp.broadcast_to(xr[1:2, :], (NH, CBLK))], axis=0)
        lhs = jnp.where(diag, xb, 0.0).astype(bf16)
        return acc + _dot(lhs, wqb_v[pl.ds(j * CBLK, CBLK), :])

    def qabs_block(j, q64):
        r = _dot_nt(q64, wuk_v[pl.ds(j * CBLK, CBLK), :])
        return _dot_nt(jnp.where(diag, r, 0.0).astype(bf16), E0)

    def latent_attention_half(b, hf, qabs):
        rows = pl.ds(hf * HALF, HALF)
        _wait_all(c_v.at[b, rows], wsem.at[S_C + 2 * b + hf])
        c = c_v[b, rows, :]
        s = _dot_nt(qabs[b * NH:(b + 1) * NH], c) * SCALE
        m = jnp.max(s, axis=1, keepdims=True)
        p = jnp.exp(s - m)
        return m, jnp.sum(p, axis=1, keepdims=True), _dot(p.astype(bf16), c)

    def merge(h0, h1):
        (m0, l0, c0), (m1, l1, c1) = h0, h1
        m = jnp.maximum(m0, m1)
        a0, a1 = jnp.exp(m0 - m), jnp.exp(m1 - m)
        return (a0 * c0 + a1 * c1) / (a0 * l0 + a1 * l1)

    def ctx_block(j, ctxl, acc):
        e = _dot(ctxl[:, j * DH:(j + 1) * DH], E0)
        lhs = jnp.where(diag, e, 0.0).astype(bf16)
        return acc + _dot(lhs, wuv_v[pl.ds(j * CBLK, CBLK), :])

    _wait_all(wqb_v, wsem.at[S_WQB])
    _wait_all(wuk_v, wsem.at[S_WUK])
    q64 = jnp.zeros((NBH, DH), jnp.float32)
    for j in range(4):
        q64 = q_block(j, q64)
    q64 = q64.astype(bf16)
    issue_c(1)
    qparts = [qabs_block(0, q64), qabs_block(1, q64)]
    issue_c(2)
    qparts += [qabs_block(2, q64), qabs_block(3, q64)]
    qabs = jnp.concatenate(qparts, axis=1).astype(bf16)
    issue_c(3)
    p00 = latent_attention_half(0, 0, qabs)
    issue_wq_wuv(0)
    p10 = latent_attention_half(1, 0, qabs)
    issue_wq_wuv(1)
    p01 = latent_attention_half(0, 1, qabs)
    issue_kv(0, 0, 0, PER // 2)
    p11 = latent_attention_half(1, 1, qabs)
    ctxl = jnp.concatenate([merge(p00, p01), merge(p10, p11)], axis=0).astype(bf16)
    issue_kv(0, 0, PER // 2, PER)
    _wait_all(wuv_v, wsem.at[S_WUV])
    _wait_all(wq_v, wsem.at[S_WQ])
    ctx = jnp.zeros((NBH, DH), jnp.float32)
    for j in range(2):
        ctx = ctx_block(j, ctxl, ctx)
    issue_kv(1, 1, 0, PER // 2)
    for j in range(2, 4):
        ctx = ctx_block(j, ctxl, ctx)
    rowh = jax.lax.broadcasted_iota(jnp.int32, (ROWS, DH), 0)
    for h in range(NH):
        cb_v[:, h * DH:(h + 1) * DH] = jnp.where(
            rowh == 0, ctx[h:h + 1, :], jnp.where(rowh == 1, ctx[NH + h:NH + h + 1, :], 0.0)).astype(bf16)
    issue_kv(1, 1, PER // 2, PER)
    qa = _dot(x16, wq_v[...]).astype(bf16)
    for h in range(NH):
        q_v[h] = qa[:, h * DH:(h + 1) * DH]
    g = jax.nn.sigmoid(jnp.sum(xf * g_v[...].reshape(1, DM).astype(jnp.float32), axis=1, keepdims=True))
    issue_kv(2, 2)

    def project(u, r0, nr, sem_a, sem_b):
        sl = (pl.ds(4 * u, 4), pl.ds(r0, nr))
        _wait_all(wo_v.at[sl], sem_a)
        _wait_all(wob_v.at[sl], sem_b)
        cols = [pl.ds(2048 * u + 512 * s + r0, nr) for s in range(4)]
        rowp = jax.lax.broadcasted_iota(jnp.int32, (ROWS, 4 * nr), 0)
        la = jnp.where(rowp == 0, jnp.concatenate([oa_v[0, :, c] for c in cols], axis=1),
                       jnp.where(rowp == 1, jnp.concatenate([oa_v[1, :, c] for c in cols], axis=1),
                                 jnp.zeros((), bf16)))
        lb = jnp.concatenate([cb_v[:, c] for c in cols], axis=1)
        return _dot(la, wo_v[sl].reshape(4 * nr, DM)), _dot(lb, wob_v[sl].reshape(4 * nr, DM))

    def head(i, carry):
        h = i % NH
        b = i // NH
        slot = i % RING
        _wait_all(kbuf.at[slot], ksem.at[slot])
        s = _dot_nt(q_v[h], kbuf[slot]) * SCALE
        m = jnp.max(s, axis=1, keepdims=True)
        p = jnp.exp(s - m)
        l = jnp.sum(p, axis=1, keepdims=True)
        _wait_all(vbuf.at[slot], vsem.at[slot])
        o = _dot(p.astype(bf16), vbuf[slot])
        oa_v[b, :, pl.ds(pl.multiple_of(h * DH, DH), DH)] = (o / l).astype(bf16)

        @pl.when(i + RING < NBH)
        def _():
            issue_kv(i + RING, slot)

        @pl.when(i == NBH - RING)
        def _():
            issue_wo_wob0()

        @pl.when(i == NBH - RING + 1)
        def _():
            _issue(wo_chunks(wo_hbm, wo_v, 1), psem.at[0], wo_chunks(wob_hbm, wob_v, 1), psem.at[1], 0, LAST_CUT)
            acc_v[0], acc_v[1] = project(0, 0, 512, wsem.at[S_WO], wsem.at[S_WOB])
            _issue(wo_chunks(wo_hbm, wo_v, 1), psem.at[2], wo_chunks(wob_hbm, wob_v, 1), psem.at[3], LAST_CUT, PER)
        return carry

    jax.lax.fori_loop(0, NBH, head, 0)

    acc_a, acc_b = acc_v[0], acc_v[1]
    for p, (c0, c1) in enumerate(((0, LAST_CUT), (LAST_CUT, PER))):
        da, db = project(1, c0 * 32, (c1 - c0) * 32, psem.at[2 * p], psem.at[2 * p + 1])
        acc_a, acc_b = acc_a + da, acc_b + db
    out_ref[...] = (g * acc_a[0:NB] + (1.0 - g) * acc_b[0:NB]).astype(out_ref.dtype)


@jax.jit
def pallas_gated_mix__mha_block_cached__compressed_kv_cla__decode_kernel(
    A_x: jax.Array,
    A_k_cache: jax.Array,
    A_v_cache: jax.Array,
    A_wq: jax.Array,
    A_wo: jax.Array,
    B_x: jax.Array,
    B_c_kv: jax.Array,
    B_w_q: jax.Array,
    B_w_uk: jax.Array,
    B_w_uv: jax.Array,
    B_w_o: jax.Array,
    gate_w: jax.Array,
):
    del B_x
    bf = jnp.bfloat16
    hbm = pl.BlockSpec(memory_space=pl.ANY)
    out = pl.pallas_call(
        _kernel,
        in_specs=[hbm] * 11,
        out_specs=pl.BlockSpec(memory_space=pltpu.VMEM),
        out_shape=jax.ShapeDtypeStruct((NB, DM), bf),
        scratch_shapes=[
            pltpu.VMEM((RING, SK, DH), bf),
            pltpu.VMEM((RING, SK, DH), bf),
            pltpu.VMEM((DM, NH * DH), bf),
            pltpu.VMEM((8, 512, DM), bf),
            pltpu.VMEM((NB, SK, DC), bf),
            pltpu.VMEM((DM * NH, DH), bf),
            pltpu.VMEM((DC * NH, DH), bf),
            pltpu.VMEM((DC * NH, DH), bf),
            pltpu.VMEM((8, 512, DM), bf),
            pltpu.VMEM((NB, DM), bf),
            pltpu.VMEM((DM,), bf),
            pltpu.VMEM((NH, ROWS, DH), bf),
            pltpu.VMEM((NB, ROWS, NH * DH), bf),
            pltpu.VMEM((ROWS, NH * DH), bf),
            pltpu.VMEM((DH, CBLK), bf),
            pltpu.VMEM((2, ROWS, DM), jnp.float32),
            pltpu.SemaphoreType.DMA((RING,)),
            pltpu.SemaphoreType.DMA((RING,)),
            pltpu.SemaphoreType.DMA((N_WSEM,)),
            pltpu.SemaphoreType.DMA((4,)),
        ],
        compiler_params=pltpu.CompilerParams(vmem_limit_bytes=100 * 1024 * 1024),
    )(
        A_x.reshape(NB, DM),
        gate_w,
        A_k_cache.reshape(NBH, SK, DH),
        A_v_cache.reshape(NBH, SK, DH),
        A_wq,
        A_wo,
        B_c_kv,
        B_w_q.reshape(DM * NH, DH),
        B_w_uk.reshape(DC * NH, DH),
        B_w_uv.reshape(DC * NH, DH),
        B_w_o.reshape(NH * DH, DM),
    )
    return out.reshape(NB, 1, DM)
```
